```python
import jax
import jax.numpy as jnp

def _softmax(x, axis=-1):
    return jax.nn.softmax(x, axis=axis)

def _gelu(x):
    return jax.nn.gelu(x, approximate=True)

def _silu(x):
    return jax.nn.silu(x)

def _sigmoid(x):
    return jax.nn.sigmoid(x)

def _layernorm(x, axis=-1, eps=1e-05):
    m = jnp.mean(x, axis=axis, keepdims=True)
    v = jnp.var(x, axis=axis, keepdims=True)
    return (x - m) / jnp.sqrt(v + eps)

def _scatter_add(tgt, idx, src, axis=0):
    return tgt.at[idx].add(src)

def _segment_sum(src, seg, n):
    return jax.ops.segment_sum(src, seg, n)

class _Rng:

    def __init__(self, key):
        self._k = key

    def _next(self):
        self._k, sub = jax.random.split(self._k)
        return sub

    def normal(self, shape):
        return jax.random.normal(self._next(), shape, dtype=jnp.bfloat16)

    def randint(self, lo, hi, shape):
        return jax.random.randint(self._next(), shape, lo, hi, dtype=jnp.int32)

    def uniform(self, shape, lo=0.0, hi=1.0):
        return jax.random.uniform(self._next(), shape, jnp.bfloat16, lo, hi)

    def permutation(self, n):
        return jax.random.permutation(self._next(), n)
kernel_name = 'adaLN_cond__ssm_conv_h3__glu_gated_reglu__prompt'

def setup_inputs():
    _rng = _Rng(jax.random.key(int.from_bytes(__import__("os").urandom(4), "little")))
    _w = lambda a: (lambda t: t.astype(jnp.bfloat16) if jnp.issubdtype(t.dtype, jnp.floating) else t)(jnp.asarray(a))

    def _A_setup():
        B, S, D = (1, 2048, 640)
        ks = 4
        return {'q': _w((lambda *s: _rng.normal(s) * 0.05)(B, S, D)), 'k': _w((lambda *s: _rng.normal(s) * 0.05)(B, S, D)), 'v': _w((lambda *s: _rng.normal(s) * 0.05)(B, S, D)), 'shift_k': _w((lambda *s: _rng.normal(s) * 0.05)(D, ks) * 0.5), 'ssm_k': _w((lambda *s: _rng.normal(s) * 0.05)(D, S) * (1.0 / S ** 0.5)), 'ssm_D': _w((lambda *s: _rng.normal(s) * 0.05)(D))}
    _A_in = _A_setup()

    def _B_setup():
        B, S, D, F = (1, 2048, 640, 1536)
        return {'x': _w((lambda *s: _rng.normal(s) * 0.05)(B, S, D)), 'W_gate': _w((lambda *s: _rng.normal(s) * 0.05)(D, F) * (2.0 / D) ** 0.5), 'W_up': _w((lambda *s: _rng.normal(s) * 0.05)(D, F) * (2.0 / D) ** 0.5), 'W_down': _w((lambda *s: _rng.normal(s) * 0.05)(F, D) * (1.0 / F) ** 0.5)}
    _B_in = _B_setup()
    return {'A_q': _A_in['q'], 'A_k': _A_in['k'], 'A_v': _A_in['v'], 'A_shift_k': _A_in['shift_k'], 'A_ssm_k': _A_in['ssm_k'], 'A_ssm_D': _A_in['ssm_D'], 'B_x': _B_in['x'], 'B_W_gate': _B_in['W_gate'], 'B_W_up': _B_in['W_up'], 'B_W_down': _B_in['W_down'], 'c': _w((lambda *s: _rng.normal(s) * 0.05)(1, 640)), 'w_mod': _w((lambda *s: _rng.normal(s) * 0.05)(640, 6 * 640) * 640 ** (-0.5))}

def reference(A_q, A_k, A_v, A_shift_k, A_ssm_k, A_ssm_D, B_x, B_W_gate, B_W_up, B_W_down, c, w_mod):

    def _A_ref(q, k, v, shift_k, ssm_k, ssm_D):
        B, S, D = q.shape
        ks = shift_k.shape[-1]
        k_pad = jnp.pad(k, ((0, 0), (ks - 1, 0), (0, 0)))
        k_shift = jnp.zeros_like(k)
        for t in range(ks):
            k_shift = k_shift + k_pad[:, t:t + S, :] * shift_k[:, ks - 1 - t][None, None, :]
        kv = k_shift * v
        L = 2 * S
        kv_pad = jnp.pad(kv, ((0, 0), (0, S), (0, 0)))
        kf_pad = jnp.pad(ssm_k, ((0, 0), (0, S)))
        kv_f = (lambda x, axes=(-2, -1): jnp.fft.rfft2(x.astype(jnp.float32), axes=axes))(kv_pad[:, None, :, :], axes=(1, 2))
        kf_f = (lambda x, axes=(-2, -1): jnp.fft.rfft2(x.astype(jnp.float32), axes=axes))(kf_pad[:, None, :], axes=(1, 2))
        kf_f = (lambda x, *d: x.transpose(*d))(kf_f, 1, 2, 0)
        y_f = kv_f * kf_f[None, :, :, :]
        y = (lambda x, s, axes=(-2, -1): jnp.fft.irfft2(x, s=s, axes=axes).astype(jnp.bfloat16))(y_f, (1, L), axes=(1, 2))[:, 0, :S, :]
        y = y + kv * ssm_D[None, None, :]
        return q * y

    def _B_ref(x, W_gate, W_up, W_down):
        gate = jnp.einsum('bsd,df->bsf', x, W_gate)
        up = jnp.einsum('bsd,df->bsf', x, W_up)
        gate = gate * (lambda x, dt: x.astype(dt))(gate > 0, gate.dtype)
        h = gate * up
        return jnp.einsum('bsf,fd->bsd', h, W_down)
    x = A_q
    mod = (_silu(c) @ w_mod).reshape(c.shape[0], 6, 1, -1)
    sa, ca, ga, sb, cb, gb = (mod[:, 0].copy(), mod[:, 1].copy(), mod[:, 2].copy(), mod[:, 3].copy(), mod[:, 4].copy(), mod[:, 5].copy())
    h = _layernorm(x, axis=-1) * (1 + ca) + sa
    x = x + ga * _A_ref(h, A_k, A_v, A_shift_k, A_ssm_k, A_ssm_D)
    h = _layernorm(x, axis=-1) * (1 + cb) + sb
    x = x + gb * _B_ref(h, B_W_gate, B_W_up, B_W_down)
    return x
```

```python
import contextlib
import numpy as np
import ml_dtypes
import jax
import jax.numpy as jnp
import jax.experimental.pallas as pl
import jax.experimental.pallas.tpu as pltpu

C = 128
L = 128
GS = 4
f32 = jnp.float32
bf16 = jnp.bfloat16


def _dft_mats():
    n = np.arange(C)[None, :].astype(np.float64)
    k = np.arange(C)[:, None].astype(np.float64)
    th = np.pi * (2 * k + 1) * n / (2 * C)
    F = np.concatenate([np.cos(th), -np.sin(th)], axis=0)
    G = np.concatenate([np.cos(th).T, -np.sin(th).T], axis=1) / C
    cast = lambda a: a.astype(np.float32).astype(ml_dtypes.bfloat16)
    return cast(F), cast(G)


_F, _G = _dft_mats()

CFG = dict(CH=1, ICH=4, BM=256, BF=512, WB=512, RB=16, scopes=False, il=True, jb2=3, jb3=3, pmode=1, wguard='when')


def scope(name):
    return jax.named_scope(name) if CFG['scopes'] else contextlib.nullcontext()


def interleave(*lists):
    lists = [l for l in lists if l]
    items = []
    for li, l in enumerate(lists):
        for i, t in enumerate(l):
            items.append(((i + 0.5) / len(l) if CFG['il'] else li, li, i, t))
    items.sort(key=lambda x: x[:3])
    for it in items:
        it[3]()


def kernel(q_hbm, k_hbm, v_hbm, shT_hbm, ssm_hbm, D_hbm, wg_hbm, wu_hbm, wd_hbm, c_hbm, wm_hbm, F_hbm, G_hbm,
           o_hbm,
           shT_ref, D_ref, c_ref, F_ref, G_ref,
           q_s, k_s, v_s, ssm_s, wg_s, wu_s, wd_s, wm_s, kf_s, X_s, K_s, Z_s, y_s, x1_s, h2_s, o_s, mod_s,
           sems):
    S, D = k_s.shape
    Fd = wg_s.shape[1]
    n = S // C
    NL = D // L
    CH, ICH, BM, BF, WB, RB = [CFG[k] for k in ('CH', 'ICH', 'BM', 'BF', 'WB', 'RB')]
    SC = CH * C
    nsc = S // SC
    nwb = Fd // WB
    nq = S // BM
    off = {}
    tot = 0
    for nm, cnt in (('small', 5), ('k', nsc), ('v', nsc), ('ssm', nsc), ('q', nq), ('wm', 6), ('wg', nwb), ('wu', nwb),
                    ('wd', nwb), ('o', nq)):
        off[nm] = tot
        tot += cnt
    sem = lambda nm, i: sems.at[off[nm] + i]
    mo = lambda r, m: r if isinstance(r, int) else pl.multiple_of(r, m)

    def cp_k(i): return pltpu.make_async_copy(k_hbm.at[pl.ds(mo(i * SC, SC), SC), :], k_s.at[pl.ds(mo(i * SC, SC), SC), :], sem('k', i))
    def cp_v(i): return pltpu.make_async_copy(v_hbm.at[pl.ds(mo(i * SC, SC), SC), :], v_s.at[pl.ds(mo(i * SC, SC), SC), :], sem('v', i))
    def cp_ssm(i): return pltpu.make_async_copy(ssm_hbm.at[:, pl.ds(mo(i * SC, SC), SC)], ssm_s.at[:, pl.ds(mo(i * SC, SC), SC)], sem('ssm', i))
    def cp_q(i): return pltpu.make_async_copy(q_hbm.at[pl.ds(mo(i * BM, BM), BM), :], q_s.at[pl.ds(mo(i * BM, BM), BM), :], sem('q', i))
    def cp_wm(i): return pltpu.make_async_copy(wm_hbm.at[:, pl.ds(i * D, D)], wm_s.at[:, pl.ds(i * D, D)], sem('wm', i))
    def cp_wg(i): return pltpu.make_async_copy(wg_hbm.at[:, pl.ds(i * WB, WB)], wg_s.at[:, pl.ds(i * WB, WB)], sem('wg', i))
    def cp_wu(i): return pltpu.make_async_copy(wu_hbm.at[:, pl.ds(i * WB, WB)], wu_s.at[:, pl.ds(i * WB, WB)], sem('wu', i))
    def cp_wd(i): return pltpu.make_async_copy(wd_hbm.at[pl.ds(i * WB, WB), :], wd_s.at[pl.ds(i * WB, WB), :], sem('wd', i))
    def cp_o(i): return pltpu.make_async_copy(o_s.at[pl.ds(mo(i * BM, BM), BM), :], o_hbm.at[pl.ds(mo(i * BM, BM), BM), :], sem('o', i))
    small = [pltpu.make_async_copy(a, b, sem('small', i)) for i, (a, b) in enumerate(
        ((F_hbm, F_ref), (shT_hbm, shT_ref), (D_hbm, D_ref), (c_hbm, c_ref), (G_hbm, G_ref)))]

    with scope("issue"):
        cp_k(0).start(); cp_v(0).start()
        small[0].start(); small[1].start(); small[2].start()
        cp_ssm(0).start()
        small[3].start(); small[4].start()
        for i in range(1, nsc):
            cp_k(i).start(); cp_v(i).start(); cp_ssm(i).start()
        for i in CFG.get('wm_order', (1, 0, 2, 4, 3)):
            cp_wm(i).start()
        cp_q(0).start()
        for i in range(nwb):
            cp_wg(i).start(); cp_wu(i).start()
            if i == 0:
                cp_q(1).start()
            cp_wd(i).start()
        cp_q(2).start()
        cp_wm(5).start()
        for i in range(3, nq):
            cp_q(i).start()

    for l in range(NL):
        kf_s[l, 0:8, :] = jnp.zeros((8, L), f32)

    def fwd_chunk(a, shT, first, Dv=None):
        r0 = mo(a * C, C)
        kk = k_s[pl.ds(r0, C), :].astype(f32)
        for l in range(NL):
            kf_s[l, pl.ds(r0 + 8, C), :] = kk[:, l * L:(l + 1) * L]
        for l in range(NL):
            ls = slice(l * L, (l + 1) * L)
            Kf = jax.lax.dot_general(F_ref[...], ssm_s[ls, pl.ds(r0, C)], (((1,), (1,)), ((), ())),
                                     preferred_element_type=f32)
            if first:
                K_s[a, 0:C, ls] = Kf[0:C] + Dv[:, ls]
                K_s[a, C:, ls] = Kf[C:]
            else:
                K_s[a, :, ls] = Kf
            ks = kf_s[l, pl.ds(r0 + 8, C), :] * shT[0:1, ls]
            for j in range(1, 4):
                ks = ks + kf_s[l, pl.ds(r0 + 8 - j, C), :] * shT[j:j + 1, ls]
            kv = (ks * v_s[pl.ds(r0, C), ls].astype(f32)).astype(bf16)
            X_s[a, :, ls] = jnp.dot(F_ref[...], kv, preferred_element_type=f32)

    def t_mac(g, r0, l, Rr, jlo, jhi):
        a0 = GS * g

        def run():
            rre = pl.ds(mo(r0, Rr), Rr)
            rim = pl.ds(mo(r0 + C, Rr), Rr)
            ls = slice(l * L, (l + 1) * L)
            acc = [None] * GS
            kc = {}

            def getk(dl):
                if dl not in kc:
                    kr = K_s[dl, rre, ls]
                    ki = K_s[dl, rim, ls]
                    kc[dl] = (kr, ki, kr + ki)
                return kc[dl]

            for j in range(jlo, jhi):
                xr = X_s[j, rre, ls]
                xi = X_s[j, rim, ls]
                xs = xr + xi
                for t in range(GS):
                    dl = a0 + t - j
                    if dl < 0:
                        continue
                    kk = getk(dl)
                    terms = (kk[0] * xr, kk[1] * xi, kk[2] * xs)
                    acc[t] = terms if acc[t] is None else tuple(a + b for a, b in zip(acc[t], terms))
            for t in range(GS):
                if acc[t] is None:
                    continue
                P, Q, Rs = acc[t]
                yr, yi = P - Q, Rs - P - Q
                if jlo > 0:
                    yr = yr + Z_s[a0 + t, rre, ls]
                    yi = yi + Z_s[a0 + t, rim, ls]
                Z_s[a0 + t, rre, ls] = yr
                Z_s[a0 + t, rim, ls] = yi
        return run

    def mac_tasks(g, r_base, nrows, Rr, jb=None):
        out = []
        jend = GS * g + GS
        jb = jb or jend
        for dr in range(0, nrows, Rr):
            for l in range(NL):
                for j0 in range(0, jend, jb):
                    out.append(t_mac(g, r_base + dr, l, Rr, j0, min(j0 + jb, jend)))
        return out

    def mac_loop(g):
        def body(i, _):
            interleave(mac_tasks(g, i * 16, 16, 16))
            return 0
        jax.lax.fori_loop(0, C // 16, body, 0)

    row = jax.lax.broadcasted_iota(jnp.int32, (C, L), 0)

    def t_inv(a, l, first):
        def run():
            ls = slice(l * L, (l + 1) * L)
            zr = Z_s[a, 0:C, ls]
            zi = Z_s[a, C:, ls]
            if not first:
                sgn = jnp.where((row & 1) == 0, 1.0, -1.0).astype(f32)
                zr = zr - sgn * Z_s[a - 1, C:, ls]
                zi = zi + sgn * Z_s[a - 1, 0:C, ls]
            w = jnp.concatenate([zr, zi], axis=0).astype(bf16)
            y_s[pl.ds(mo(a * C, C), C), ls] = jnp.dot(G_ref[...], w, preferred_element_type=f32)
        return run

    def inv_tasks(g):
        return [t_inv(g * GS + t, l, g == 0 and t == 0) for t in range(GS) for l in range(NL)]

    def t_post(r_dst, r_src, part):
        def run():
            rep = lambda i: jnp.concatenate([mod_s[i]] * (RB // 8), axis=0)
            if part in (0, 1):
                q = q_s[pl.ds(r_src, RB), :].astype(f32)
                m = jnp.mean(q, axis=-1, keepdims=True)
                xc = q - m
                r = jax.lax.rsqrt(jnp.mean(xc * xc, axis=-1, keepdims=True) + 1e-5)
                hg = (xc * r) * rep(0) + rep(1)
                x1 = hg * y_s[pl.ds(r_src, RB), :] + q
                x1_s[pl.ds(r_dst, RB), :] = x1
            if part == 2:
                x1 = x1_s[pl.ds(r_dst, RB), :]
            if part in (0, 2):
                m2 = jnp.mean(x1, axis=-1, keepdims=True)
                xc2 = x1 - m2
                r2 = jax.lax.rsqrt(jnp.mean(xc2 * xc2, axis=-1, keepdims=True) + 1e-5)
                h2_s[pl.ds(r_dst, RB), :] = ((xc2 * r2) * rep(2) + rep(3)).astype(bf16)
        return run

    def post_tasks(r_dst, r_src):
        out = []
        for t in range(BM // RB):
            a, b = mo(r_dst + t * RB, RB), mo(r_src + t * RB, RB)
            if CFG['pmode'] == 0:
                out.append(t_post(a, b, 0))
            else:
                out.append(t_post(a, b, 1))
                out.append(t_post(a, b, 2))
        return out

    def silu_c():
        cc = c_ref[...].astype(f32)
        return jnp.broadcast_to((cc * jax.nn.sigmoid(cc)).astype(bf16), (16, D))

    def ffn_iter(i, guard, others):
        r0 = mo(i * BM, BM)
        fs = {'h2': h2_s[pl.ds(r0, BM), :]}
        tasks = []

        def guarded(fn):
            if guard is None:
                return
            pl.when(guard)(fn)

        def t_gu(f):
            def run():
                def w():
                    for b in range(f * BF // WB, (f + 1) * BF // WB):
                        cp_wg(b).wait(); cp_wu(b).wait()
                    if f == 0:
                        cp_wd(0).wait()
                if f > 0:
                    guarded(w)
                h2 = fs['h2']
                g = jnp.dot(h2, wg_s[:, f * BF:(f + 1) * BF], preferred_element_type=f32)
                u = jnp.dot(h2, wu_s[:, f * BF:(f + 1) * BF], preferred_element_type=f32)
                fs['act'] = (jnp.maximum(g, 0.0) * u).astype(bf16)
            return run

        def t_d(f):
            def run():
                if f > 0:
                    guarded(lambda: [cp_wd(b).wait() for b in range(f * BF // WB, (f + 1) * BF // WB)] and None)
                d = jnp.dot(fs['act'], wd_s[f * BF:(f + 1) * BF, :], preferred_element_type=f32)
                fs['acc'] = d if f == 0 else fs['acc'] + d
            return run

        for f in range(Fd // BF):
            tasks.append(t_gu(f))
            tasks.append(t_d(f))
        nxt = mo(jnp.minimum(r0 + BM, S - BM), BM)
        interleave(tasks, *others, post_tasks(r0 + BM, nxt))
        if guard is not None:
            @pl.when(guard)
            def _():
                cp_wm(5).wait()
                mod_s[4] = jnp.dot(silu_c(), wm_s[:, 5 * D:6 * D], preferred_element_type=f32)[0:8]
                cp_q(2).wait()
        gbv = jnp.concatenate([mod_s[4]] * (BM // 8), axis=0)
        o_s[pl.ds(r0, BM), :] = (x1_s[pl.ds(r0, BM), :] + gbv * fs['acc']).astype(o_s.dtype)
        cp_o(i).start()

    with scope("fwd0"):
        cp_k(0).wait(); cp_v(0).wait(); small[0].wait(); small[1].wait(); small[2].wait(); cp_ssm(0).wait()
        shT = shT_ref[...].astype(f32)
        Dv = D_ref[...].astype(f32).reshape(1, D)
        for t in range(CH):
            fwd_chunk(t, shT, t == 0, Dv)
    with scope("fwd"):
        def fbody(i, _):
            cp_k(i).wait(); cp_v(i).wait(); cp_ssm(i).wait()
            for t in range(CH):
                fwd_chunk(i * CH + t, shT, False)
            return 0
        jax.lax.fori_loop(1, nsc, fbody, 0)
    with scope("mac0"):
        mac_loop(0)
    with scope("inv0"):
        small[4].wait()
        interleave(inv_tasks(0))
    with scope("mac1"):
        mac_loop(1)
    with scope("mod"):
        small[3].wait()
        sc8 = silu_c()
        mods = [None] * 5
        for i in CFG.get('wm_order', (1, 0, 2, 4, 3)):
            cp_wm(i).wait()
            mods[i] = jnp.dot(sc8, wm_s[:, i * D:(i + 1) * D], preferred_element_type=f32)[0:8]
        sa, ca, ga, sb, cb = mods
        mod_s[0] = (1.0 + ca) * ga
        mod_s[1] = sa * ga
        mod_s[2] = 1.0 + cb
        mod_s[3] = sb
    with scope("inv1_post0"):
        cp_q(0).wait()
        interleave(inv_tasks(1), post_tasks(0, 0))
    with scope("wW"):
        cp_q(1).wait()
        for b in range(BF // WB):
            cp_wg(b).wait(); cp_wu(b).wait(); cp_wd(b).wait()
    with scope("A1"):
        def bodyA1(i, _):
            ffn_iter(i, i == 0, [mac_tasks(2, i * 64, 64, 8, CFG['jb2'])])
            return 0
        jax.lax.fori_loop(0, 2, bodyA1, 0)
    with scope("inv2"):
        interleave(inv_tasks(2))
        for i in range(3, nq):
            cp_q(i).wait()
    with scope("A2"):
        def bodyA2(i, _):
            ffn_iter(i, None, [mac_tasks(3, (i - 2) * 64, 64, 8, CFG['jb3'])])
            return 0
        jax.lax.fori_loop(2, 4, bodyA2, 0)
    with scope("inv3"):
        interleave(inv_tasks(3))
    with scope("B"):
        def bodyB(i, _):
            ffn_iter(i, None, [])
            return 0
        jax.lax.fori_loop(4, nq, bodyB, 0)
    with scope("drain"):
        for i in range(nq):
            cp_o(i).wait()


@jax.jit
def pallas_adaLN_cond__ssm_conv_h3__glu_gated_reglu__prompt_kernel(A_q, A_k, A_v, A_shift_k, A_ssm_k, A_ssm_D, B_x, B_W_gate, B_W_up, B_W_down, c, w_mod):
    _, S, D = A_q.shape
    Fd = B_W_gate.shape[1]
    n = S // C
    BM = CFG['BM']
    nwb = Fd // CFG['WB']
    nsc = n // CFG['CH']
    any_ = pl.BlockSpec(memory_space=pl.ANY)
    V = pltpu.VMEM
    dma = pltpu.SemaphoreType.DMA
    out = pl.pallas_call(
        kernel,
        out_shape=jax.ShapeDtypeStruct((S, D), A_q.dtype),
        in_specs=[any_] * 13,
        out_specs=any_,
        scratch_shapes=[V((4, D), bf16), V((D,), bf16), V((1, D), bf16), V((2 * C, C), bf16), V((C, 2 * C), bf16),
                        V((S, D), bf16), V((S, D), bf16), V((S, D), bf16), V((D, S), bf16),
                        V((D, Fd), bf16), V((D, Fd), bf16), V((Fd, D), bf16), V((D, 6 * D), bf16),
                        V((D // L, S + 8, L), f32), V((n, 2 * C, D), f32), V((n, 2 * C, D), f32),
                        V((n, 2 * C, D), f32), V((S, D), f32), V((S + BM, D), f32),
                        V((S + BM, D), bf16), V((S, D), bf16),
                        V((5, 8, D), f32),
                        dma((5 + 3 * nsc + 6 + 3 * nwb + 2 * (S // BM),))],
        compiler_params=pltpu.CompilerParams(vmem_limit_bytes=120 * 1024 * 1024, flags=CFG.get("flags") or None),
    )(A_q[0], A_k[0], A_v[0], A_shift_k.T, A_ssm_k, A_ssm_D, B_W_gate, B_W_up, B_W_down, c, w_mod,
      jnp.asarray(_F), jnp.asarray(_G))
    return out[None]
```

```python
import contextlib
import numpy as np
import ml_dtypes
import jax
import jax.numpy as jnp
import jax.experimental.pallas as pl
import jax.experimental.pallas.tpu as pltpu

C = 128
L = 128
GS = 4
f32 = jnp.float32
bf16 = jnp.bfloat16


def _dft_mats():
    n = np.arange(C)[None, :].astype(np.float64)
    k = np.arange(C)[:, None].astype(np.float64)
    th = np.pi * (2 * k + 1) * n / (2 * C)
    F = np.concatenate([np.cos(th), -np.sin(th)], axis=0)
    G = np.concatenate([np.cos(th).T, -np.sin(th).T], axis=1) / C
    cast = lambda a: a.astype(np.float32).astype(ml_dtypes.bfloat16)
    return cast(F), cast(G)


_F, _G = _dft_mats()

CFG = dict(CH=1, ICH=4, BM=256, BF=512, WB=512, RB=8, scopes=False, il=True, jb2=2, jb3=3, pmode=1, npre=8, wmode=1)


def scope(name):
    return jax.named_scope(name) if CFG['scopes'] else contextlib.nullcontext()


def interleave(*lists):
    lists = [l for l in lists if l]
    items = []
    for li, l in enumerate(lists):
        for i, t in enumerate(l):
            items.append(((i + 0.5) / len(l) if CFG['il'] else li, li, i, t))
    items.sort(key=lambda x: x[:3])
    for it in items:
        it[3]()


def kernel(q_hbm, k_hbm, v_hbm, shT_hbm, ssm_hbm, D_hbm, wg_hbm, wu_hbm, wd_hbm, c_hbm, wm_hbm, F_hbm, G_hbm,
           o_hbm,
           shT_ref, D_ref, c_ref, F_ref, G_ref,
           q_s, k_s, v_s, ssm_s, wg_s, wu_s, wd_s, wm_s, kf_s, X_s, K_s, Z_s, y_s, x1_s, h2_s, o_s, mod_s,
           sems):
    S, D = k_s.shape
    Fd = wg_s.shape[1]
    n = S // C
    NL = D // L
    CH, ICH, BM, BF, WB, RB = [CFG[k] for k in ('CH', 'ICH', 'BM', 'BF', 'WB', 'RB')]
    SC = CH * C
    nsc = S // SC
    nwb = Fd // WB
    nq = S // BM
    off = {}
    tot = 0
    for nm, cnt in (('small', 5), ('k', nsc), ('v', nsc), ('ssm', nsc), ('q', nq), ('wm', 6), ('wg', nwb), ('wu', nwb),
                    ('wd', nwb), ('o', nq)):
        off[nm] = tot
        tot += cnt
    sem = lambda nm, i: sems.at[off[nm] + i]
    mo = lambda r, m: r if isinstance(r, int) else pl.multiple_of(r, m)

    def cp_k(i): return pltpu.make_async_copy(k_hbm.at[pl.ds(mo(i * SC, SC), SC), :], k_s.at[pl.ds(mo(i * SC, SC), SC), :], sem('k', i))
    def cp_v(i): return pltpu.make_async_copy(v_hbm.at[pl.ds(mo(i * SC, SC), SC), :], v_s.at[pl.ds(mo(i * SC, SC), SC), :], sem('v', i))
    def cp_ssm(i): return pltpu.make_async_copy(ssm_hbm.at[:, pl.ds(mo(i * SC, SC), SC)], ssm_s.at[:, pl.ds(mo(i * SC, SC), SC)], sem('ssm', i))
    def cp_q(i): return pltpu.make_async_copy(q_hbm.at[pl.ds(mo(i * BM, BM), BM), :], q_s.at[pl.ds(mo(i * BM, BM), BM), :], sem('q', i))
    def cp_wm(i): return pltpu.make_async_copy(wm_hbm.at[:, pl.ds(i * D, D)], wm_s.at[:, pl.ds(i * D, D)], sem('wm', i))
    def cp_wg(i): return pltpu.make_async_copy(wg_hbm.at[:, pl.ds(i * WB, WB)], wg_s.at[:, pl.ds(i * WB, WB)], sem('wg', i))
    def cp_wu(i): return pltpu.make_async_copy(wu_hbm.at[:, pl.ds(i * WB, WB)], wu_s.at[:, pl.ds(i * WB, WB)], sem('wu', i))
    def cp_wd(i): return pltpu.make_async_copy(wd_hbm.at[pl.ds(i * WB, WB), :], wd_s.at[pl.ds(i * WB, WB), :], sem('wd', i))
    def cp_o(i): return pltpu.make_async_copy(o_s.at[pl.ds(mo(i * BM, BM), BM), :], o_hbm.at[pl.ds(mo(i * BM, BM), BM), :], sem('o', i))
    small = [pltpu.make_async_copy(a, b, sem('small', i)) for i, (a, b) in enumerate(
        ((F_hbm, F_ref), (shT_hbm, shT_ref), (D_hbm, D_ref), (c_hbm, c_ref), (G_hbm, G_ref)))]

    npre = CFG['npre']
    with scope("issue"):
        cp_k(0).start(); cp_v(0).start()
        small[0].start(); small[1].start(); small[2].start()
        cp_ssm(0).start()
        small[3].start(); small[4].start()
        for i in range(1, npre):
            cp_k(i).start(); cp_v(i).start(); cp_ssm(i).start()
        for i in (1, 0, 2, 4, 3):
            cp_wm(i).start()
        cp_q(0).start()
        cp_wg(0).start(); cp_wu(0).start()
        cp_q(1).start()
        mid = CFG.get('mid', True)
        for i in range(nwb):
            cp_wd(i).start()
            if mid and i == nwb - 2:
                for j in range(npre, 12):
                    cp_k(j).start(); cp_v(j).start(); cp_ssm(j).start()
            if i + 1 < nwb:
                cp_wg(i + 1).start(); cp_wu(i + 1).start()
        cp_wm(5).start()
        cp_q(2).start()
        if not mid:
            for i in range(npre, 12):
                cp_k(i).start(); cp_v(i).start(); cp_ssm(i).start()
        cp_q(3).start()
        for i in range(12, n):
            cp_k(i).start(); cp_v(i).start(); cp_ssm(i).start()
        for i in range(4, nq):
            cp_q(i).start()

    for l in range(NL):
        kf_s[l, 0:8, :] = jnp.zeros((8, L), f32)

    st = {}
    def fwd_chunk(a, shT, first, Dv=None):
        r0 = mo(a * C, C)
        kk = k_s[pl.ds(r0, C), :].astype(f32)
        for l in range(NL):
            kf_s[l, pl.ds(r0 + 8, C), :] = kk[:, l * L:(l + 1) * L]
        for l in range(NL):
            ls = slice(l * L, (l + 1) * L)
            Kf = jax.lax.dot_general(F_ref[...], ssm_s[ls, pl.ds(r0, C)], (((1,), (1,)), ((), ())),
                                     preferred_element_type=f32)
            if first:
                K_s[a, 0:C, ls] = Kf[0:C] + Dv[:, ls]
                K_s[a, C:, ls] = Kf[C:]
            else:
                K_s[a, :, ls] = Kf
            ks = kf_s[l, pl.ds(r0 + 8, C), :] * shT[0:1, ls]
            for j in range(1, 4):
                ks = ks + kf_s[l, pl.ds(r0 + 8 - j, C), :] * shT[j:j + 1, ls]
            kv = (ks * v_s[pl.ds(r0, C), ls].astype(f32)).astype(bf16)
            X_s[a, :, ls] = jnp.dot(F_ref[...], kv, preferred_element_type=f32)

    def t_mac(g, r0, l, Rr, jlo, jhi):
        a0 = GS * g

        def run():
            rre = pl.ds(mo(r0, Rr), Rr)
            rim = pl.ds(mo(r0 + C, Rr), Rr)
            ls = slice(l * L, (l + 1) * L)
            acc = [None] * GS
            kc = {}

            def getk(dl):
                if dl not in kc:
                    kr = K_s[dl, rre, ls]
                    ki = K_s[dl, rim, ls]
                    kc[dl] = (kr, ki, kr + ki)
                return kc[dl]

            for j in range(jlo, jhi):
                xr = X_s[j, rre, ls]
                xi = X_s[j, rim, ls]
                xs = xr + xi
                for t in range(GS):
                    dl = a0 + t - j
                    if dl < 0:
                        continue
                    kk = getk(dl)
                    terms = (kk[0] * xr, kk[1] * xi, kk[2] * xs)
                    acc[t] = terms if acc[t] is None else tuple(a + b for a, b in zip(acc[t], terms))
            for t in range(GS):
                if acc[t] is None:
                    continue
                P, Q, Rs = acc[t]
                yr, yi = P - Q, Rs - P - Q
                if jlo > 0:
                    yr = yr + Z_s[a0 + t, rre, ls]
                    yi = yi + Z_s[a0 + t, rim, ls]
                Z_s[a0 + t, rre, ls] = yr
                Z_s[a0 + t, rim, ls] = yi
        return run

    def mac_tasks(g, r_base, nrows, Rr, jb=None):
        out = []
        jend = GS * g + GS
        jb = jb or jend
        for dr in range(0, nrows, Rr):
            for l in range(NL):
                for j0 in range(0, jend, jb):
                    out.append(t_mac(g, r_base + dr, l, Rr, j0, min(j0 + jb, jend)))
        return out

    def mac_loop(g):
        def body(i, _):
            interleave(mac_tasks(g, i * 16, 16, 16))
            return 0
        jax.lax.fori_loop(0, C // 16, body, 0)

    row = jax.lax.broadcasted_iota(jnp.int32, (C, L), 0)

    def t_inv(a, l, first):
        def run():
            ls = slice(l * L, (l + 1) * L)
            zr = Z_s[a, 0:C, ls]
            zi = Z_s[a, C:, ls]
            if not first:
                sgn = jnp.where((row & 1) == 0, 1.0, -1.0).astype(f32)
                zr = zr - sgn * Z_s[a - 1, C:, ls]
                zi = zi + sgn * Z_s[a - 1, 0:C, ls]
            w = jnp.concatenate([zr, zi], axis=0).astype(bf16)
            y_s[pl.ds(mo(a * C, C), C), ls] = jnp.dot(G_ref[...], w, preferred_element_type=f32)
        return run

    def inv_tasks(g):
        return [t_inv(g * GS + t, l, g == 0 and t == 0) for t in range(GS) for l in range(NL)]

    def t_post(r_dst, r_src, part):
        def run():
            rep = lambda i: jnp.concatenate([mod_s[i]] * (RB // 8), axis=0)
            if part in (0, 1):
                q = q_s[pl.ds(r_src, RB), :].astype(f32)
                m = jnp.mean(q, axis=-1, keepdims=True)
                xc = q - m
                r = jax.lax.rsqrt(jnp.mean(xc * xc, axis=-1, keepdims=True) + 1e-5)
                hg = (xc * r) * rep(0) + rep(1)
                x1 = hg * y_s[pl.ds(r_src, RB), :] + q
                x1_s[pl.ds(r_dst, RB), :] = x1
            if part == 2:
                x1 = x1_s[pl.ds(r_dst, RB), :]
            if part in (0, 2):
                m2 = jnp.mean(x1, axis=-1, keepdims=True)
                xc2 = x1 - m2
                r2 = jax.lax.rsqrt(jnp.mean(xc2 * xc2, axis=-1, keepdims=True) + 1e-5)
                h2_s[pl.ds(r_dst, RB), :] = ((xc2 * r2) * rep(2) + rep(3)).astype(bf16)
        return run

    def post_tasks(r_dst, r_src):
        out = []
        for t in range(BM // RB):
            a, b = mo(r_dst + t * RB, RB), mo(r_src + t * RB, RB)
            if CFG['pmode'] == 0:
                out.append(t_post(a, b, 0))
            else:
                out.append(t_post(a, b, 1))
                out.append(t_post(a, b, 2))
        return out

    def silu_c():
        cc = c_ref[...].astype(f32)
        return jnp.broadcast_to((cc * jax.nn.sigmoid(cc)).astype(bf16), (16, D))

    def ffn_iter(i, guard, others):
        ffn_iter_(i, guard, others)

    def ffn_iter_(i, guard, others):
        r0 = mo(i * BM, BM)
        fs = {'h2': h2_s[pl.ds(r0, BM), :]}
        tasks = []

        def guarded(fn):
            if guard is not None:
                fn()

        def t_gu(f):
            def run():
                wm = CFG['wmode']
                blk = lambda ff: range(ff * BF // WB, (ff + 1) * BF // WB)
                if wm == 0 and f > 0:
                    guarded(lambda: [(cp_wg(b).wait(), cp_wu(b).wait()) for b in blk(f)] and None)
                if wm == 2 and f > 0:
                    guarded(lambda: [(cp_wg(b).wait(), cp_wu(b).wait(), cp_wd(b).wait()) for b in blk(f)] and None)
                h2 = fs['h2']
                g = jnp.dot(h2, wg_s[:, f * BF:(f + 1) * BF], preferred_element_type=f32)
                u = jnp.dot(h2, wu_s[:, f * BF:(f + 1) * BF], preferred_element_type=f32)
                fs['act'] = (jnp.maximum(g, 0.0) * u).astype(bf16)
            return run

        def t_d(f):
            def run():
                wm = CFG['wmode']
                blk = lambda ff: range(ff * BF // WB, (ff + 1) * BF // WB)
                nf = Fd // BF
                if wm == 0 and f > 0:
                    guarded(lambda: [cp_wd(b).wait() for b in blk(f)] and None)
                if wm == 1:
                    def w():
                        if f == 0:
                            cp_q(1).wait()
                        for b in blk(f):
                            cp_wd(b).wait()
                        if f + 1 < nf and not (CFG.get('mid', True) and f + 2 == nf):
                            for b in blk(f + 1):
                                cp_wg(b).wait(); cp_wu(b).wait()
                    guarded(w)
                d = jnp.dot(fs['act'], wd_s[f * BF:(f + 1) * BF, :], preferred_element_type=f32)
                fs['acc'] = d if f == 0 else fs['acc'] + d
            return run

        for f in range(Fd // BF):
            tasks.append(t_gu(f))
            tasks.append(t_d(f))
        nxt = mo(jnp.minimum(r0 + BM, S - BM), BM)
        if guard is None:
            interleave(tasks, *others, post_tasks(r0 + BM, nxt))
        else:
            tasks[0]()
            if CFG.get('mid', True):
                pt = post_tasks(r0 + BM, nxt)
                interleave(tasks[1:-2], pt)
                st['late_fwd'](npre, 12)
                for b in range((Fd - BF) // WB, nwb):
                    cp_wg(b).wait(); cp_wu(b).wait()
                interleave(tasks[-2:])
            else:
                interleave(tasks[1:], *others, post_tasks(r0 + BM, nxt))
            cp_wm(5).wait()
            mod_s[4] = jnp.dot(silu_c(), wm_s[:, 5 * D:6 * D], preferred_element_type=f32)[0:8]
        gbv = jnp.concatenate([mod_s[4]] * (BM // 8), axis=0)
        o_s[pl.ds(r0, BM), :] = (x1_s[pl.ds(r0, BM), :] + gbv * fs['acc']).astype(o_s.dtype)
        cp_o(i).start()

    with scope("fwd0"):
        cp_k(0).wait(); cp_v(0).wait(); small[0].wait(); small[1].wait(); small[2].wait(); cp_ssm(0).wait()
        shT = shT_ref[...].astype(f32)
        Dv = D_ref[...].astype(f32).reshape(1, D)
        for t in range(CH):
            fwd_chunk(t, shT, t == 0, Dv)
    with scope("fwd"):
        def fbody(i, _):
            cp_k(i).wait(); cp_v(i).wait(); cp_ssm(i).wait()
            fwd_chunk(i, shT, False)
            return 0
        jax.lax.fori_loop(1, npre, fbody, 0)

    def late_fwd(lo, hi, extra=()):
        for i in range(lo, hi):
            cp_k(i).wait(); cp_v(i).wait(); cp_ssm(i).wait()
        sh = shT_ref[...].astype(f32)
        interleave([(lambda i=i: fwd_chunk(i, sh, False)) for i in range(lo, hi)], list(extra))
    st['late_fwd'] = late_fwd
    with scope("mac0"):
        mac_loop(0)
    with scope("inv0"):
        small[4].wait()
        interleave(inv_tasks(0))
    with scope("mac1"):
        mac_loop(1)
    with scope("mod"):
        small[3].wait()
        sc8 = silu_c()
        mods = [None] * 5
        for i in CFG.get('wm_order', (1, 0, 2, 4, 3)):
            cp_wm(i).wait()
            mods[i] = jnp.dot(sc8, wm_s[:, i * D:(i + 1) * D], preferred_element_type=f32)[0:8]
        sa, ca, ga, sb, cb = mods
        mod_s[0] = (1.0 + ca) * ga
        mod_s[1] = sa * ga
        mod_s[2] = 1.0 + cb
        mod_s[3] = sb
    with scope("inv1_post0"):
        cp_q(0).wait()
        interleave(inv_tasks(1), post_tasks(0, 0))
    with scope("wW"):
        for b in range(BF // WB):
            cp_wg(b).wait(); cp_wu(b).wait()
    with scope("P0"):
        def bodyP0(i, _):
            ffn_iter(i, True, [])
            return 0
        if CFG.get('p0loop'):
            jax.lax.fori_loop(0, 1, bodyP0, 0)
        else:
            bodyP0(0, 0)
    if npre < 12 and not CFG.get('mid', True):
        with scope("fwd2"):
            late_fwd(npre, 12)
    with scope("A1"):
        cp_q(2).wait(); cp_q(3).wait()

        def bodyA1(i, _):
            ffn_iter(i, None, [mac_tasks(2, (i - 1) * 64, 64, 8, CFG['jb2'])])
            return 0
        jax.lax.fori_loop(1, 3, bodyA1, 0)
    if CFG.get('fuse23', True):
        with scope("inv2fwd3"):
            late_fwd(12, n, inv_tasks(2))
            for i in range(4, nq):
                cp_q(i).wait()
    else:
        with scope("inv2"):
            interleave(inv_tasks(2))
        with scope("fwd3"):
            late_fwd(12, n)
            for i in range(4, nq):
                cp_q(i).wait()
    with scope("A2"):
        def bodyA2(i, _):
            ffn_iter(i, None, [mac_tasks(3, (i - 3) * 64, 64, 8, CFG['jb3'])])
            return 0
        jax.lax.fori_loop(3, 5, bodyA2, 0)
    with scope("inv3"):
        interleave(inv_tasks(3))
    with scope("B"):
        def bodyB(i, _):
            ffn_iter(i, None, [])
            return 0
        jax.lax.fori_loop(5, nq, bodyB, 0)
    with scope("drain"):
        for i in range(nq):
            cp_o(i).wait()


@jax.jit
def pallas_adaLN_cond__ssm_conv_h3__glu_gated_reglu__prompt_kernel(A_q, A_k, A_v, A_shift_k, A_ssm_k, A_ssm_D, B_x, B_W_gate, B_W_up, B_W_down, c, w_mod):
    _, S, D = A_q.shape
    Fd = B_W_gate.shape[1]
    n = S // C
    BM = CFG['BM']
    nwb = Fd // CFG['WB']
    nsc = n // CFG['CH']
    any_ = pl.BlockSpec(memory_space=pl.ANY)
    V = pltpu.VMEM
    dma = pltpu.SemaphoreType.DMA
    out = pl.pallas_call(
        kernel,
        out_shape=jax.ShapeDtypeStruct((S, D), A_q.dtype),
        in_specs=[any_] * 13,
        out_specs=any_,
        scratch_shapes=[V((4, D), bf16), V((D,), bf16), V((1, D), bf16), V((2 * C, C), bf16), V((C, 2 * C), bf16),
                        V((S, D), bf16), V((S, D), bf16), V((S, D), bf16), V((D, S), bf16),
                        V((D, Fd), bf16), V((D, Fd), bf16), V((Fd, D), bf16), V((D, 6 * D), bf16),
                        V((D // L, S + 8, L), f32), V((n, 2 * C, D), f32), V((n, 2 * C, D), f32),
                        V((n, 2 * C, D), f32), V((S, D), f32), V((S + BM, D), f32),
                        V((S + BM, D), bf16), V((S, D), bf16),
                        V((5, 8, D), f32),
                        dma((5 + 3 * nsc + 6 + 3 * nwb + 2 * (S // BM),))],
        compiler_params=pltpu.CompilerParams(vmem_limit_bytes=120 * 1024 * 1024, flags=CFG.get("flags") or None),
    )(A_q[0], A_k[0], A_v[0], A_shift_k.T, A_ssm_k, A_ssm_D, B_W_gate, B_W_up, B_W_down, c, w_mod,
      jnp.asarray(_F), jnp.asarray(_G))
    return out[None]
```

```python
import contextlib
import numpy as np
import ml_dtypes
import jax
import jax.numpy as jnp
import jax.experimental.pallas as pl
import jax.experimental.pallas.tpu as pltpu

C = 128
L = 128
GS = 4
f32 = jnp.float32
bf16 = jnp.bfloat16


def _dft_mats():
    n = np.arange(C)[None, :].astype(np.float64)
    k = np.arange(C)[:, None].astype(np.float64)
    th = np.pi * (2 * k + 1) * n / (2 * C)
    F = np.concatenate([np.cos(th), -np.sin(th)], axis=0)
    G = np.concatenate([np.cos(th).T, -np.sin(th).T], axis=1) / C
    cast = lambda a: a.astype(np.float32).astype(ml_dtypes.bfloat16)
    return cast(F), cast(G)


_F, _G = _dft_mats()

CFG = dict(CH=1, ICH=4, BM=256, BF=512, WB=512, RB=8, scopes=False, il=True, jb2=2, jb3=3, pmode=1, npre=8, wmode=1, inv1late=1, osplit=1, early3=[[4, 6], [6, 8]], late3=[[0, 2], [2, 4], [8, 10], [10, 12], [12, 14], [14, 16]], big=1, midc=4)


def scope(name):
    return jax.named_scope(name) if CFG['scopes'] else contextlib.nullcontext()


def interleave(*lists):
    lists = [l for l in lists if l]
    items = []
    for li, l in enumerate(lists):
        for i, t in enumerate(l):
            items.append(((i + 0.5) / len(l) if CFG['il'] else li, li, i, t))
    items.sort(key=lambda x: x[:3])
    for it in items:
        it[3]()


def kernel(q_hbm, k_hbm, v_hbm, shT_hbm, ssm_hbm, D_hbm, wg_hbm, wu_hbm, wd_hbm, c_hbm, wm_hbm, F_hbm, G_hbm,
           o_hbm,
           shT_ref, D_ref, c_ref, F_ref, G_ref,
           q_s, k_s, v_s, ssm_s, wg_s, wu_s, wd_s, wm_s, kf_s, X_s, K_s, Z_s, y_s, x1_s, h2_s, o_s, mod_s,
           sems):
    S, D = k_s.shape
    Fd = wg_s.shape[1]
    n = S // C
    NL = D // L
    CH, ICH, BM, BF, WB, RB = [CFG[k] for k in ('CH', 'ICH', 'BM', 'BF', 'WB', 'RB')]
    SC = CH * C
    nsc = S // SC
    nwb = Fd // WB
    nq = S // BM
    off = {}
    tot = 0
    for nm, cnt in (('small', 5), ('k', nsc), ('v', nsc), ('ssm', nsc), ('q', nq), ('wm', 6), ('wg', nwb), ('wu', nwb),
                    ('wd', nwb), ('o', nq), ('o2', nq)):
        off[nm] = tot
        tot += cnt
    sem = lambda nm, i: sems.at[off[nm] + i]
    mo = lambda r, m: r if isinstance(r, int) else pl.multiple_of(r, m)

    def cp_k(i): return pltpu.make_async_copy(k_hbm.at[pl.ds(mo(i * SC, SC), SC), :], k_s.at[pl.ds(mo(i * SC, SC), SC), :], sem('k', i))
    def cp_v(i): return pltpu.make_async_copy(v_hbm.at[pl.ds(mo(i * SC, SC), SC), :], v_s.at[pl.ds(mo(i * SC, SC), SC), :], sem('v', i))
    def cp_ssm(i): return pltpu.make_async_copy(ssm_hbm.at[:, pl.ds(mo(i * SC, SC), SC)], ssm_s.at[:, pl.ds(mo(i * SC, SC), SC)], sem('ssm', i))
    def cp_multi(a, cnt):
        rs = pl.ds(a * C, cnt * C)
        return [pltpu.make_async_copy(k_hbm.at[rs, :], k_s.at[rs, :], sem('k', a)),
                pltpu.make_async_copy(v_hbm.at[rs, :], v_s.at[rs, :], sem('v', a)),
                pltpu.make_async_copy(ssm_hbm.at[:, rs], ssm_s.at[:, rs], sem('ssm', a))]

    def late_copies(lo, hi):
        if CFG['big']:
            return cp_multi(lo, hi - lo)
        return [c for j in range(lo, hi) for c in cp_multi(j, 1)]

    def cp_q(i): return pltpu.make_async_copy(q_hbm.at[pl.ds(mo(i * BM, BM), BM), :], q_s.at[pl.ds(mo(i * BM, BM), BM), :], sem('q', i))
    def cp_wm(i): return pltpu.make_async_copy(wm_hbm.at[:, pl.ds(i * D, D)], wm_s.at[:, pl.ds(i * D, D)], sem('wm', i))
    def cp_wg(i): return pltpu.make_async_copy(wg_hbm.at[:, pl.ds(i * WB, WB)], wg_s.at[:, pl.ds(i * WB, WB)], sem('wg', i))
    def cp_wu(i): return pltpu.make_async_copy(wu_hbm.at[:, pl.ds(i * WB, WB)], wu_s.at[:, pl.ds(i * WB, WB)], sem('wu', i))
    def cp_wd(i): return pltpu.make_async_copy(wd_hbm.at[pl.ds(i * WB, WB), :], wd_s.at[pl.ds(i * WB, WB), :], sem('wd', i))
    def cp_o(i): return pltpu.make_async_copy(o_s.at[pl.ds(mo(i * BM, BM), BM), :], o_hbm.at[pl.ds(mo(i * BM, BM), BM), :], sem('o', i))
    def cp_oh(i, hh):
        H = BM // 2
        rr = mo(i * BM + hh * H, H)
        return pltpu.make_async_copy(o_s.at[pl.ds(rr, H), :], o_hbm.at[pl.ds(rr, H), :], sem('o' if hh == 0 else 'o2', i))
    small = [pltpu.make_async_copy(a, b, sem('small', i)) for i, (a, b) in enumerate(
        ((F_hbm, F_ref), (shT_hbm, shT_ref), (D_hbm, D_ref), (c_hbm, c_ref), (G_hbm, G_ref)))]

    npre = CFG['npre']
    midc = CFG['midc']
    with scope("issue"):
        cp_k(0).start(); cp_v(0).start()
        small[0].start(); small[1].start(); small[2].start()
        cp_ssm(0).start()
        small[3].start(); small[4].start()
        for i in range(1, npre):
            cp_k(i).start(); cp_v(i).start(); cp_ssm(i).start()
        for i in (1, 0, 2, 4, 3):
            cp_wm(i).start()
        cp_q(0).start()
        cp_wg(0).start(); cp_wu(0).start()
        cp_q(1).start()
        mid = CFG.get('mid', True)
        for i in range(nwb):
            cp_wd(i).start()
            if mid and i == nwb - 2:
                for cpy in late_copies(npre, npre + midc):
                    cpy.start()
            if i + 1 < nwb:
                cp_wg(i + 1).start(); cp_wu(i + 1).start()
        cp_wm(5).start()
        cp_q(2).start()
        if npre + midc < 12:
            for cpy in late_copies(npre + midc, 12):
                cpy.start()
        cp_q(3).start()
        for cpy in late_copies(12, n):
            cpy.start()
        for i in range(4, nq):
            cp_q(i).start()

    for l in range(NL):
        kf_s[l, 0:8, :] = jnp.zeros((8, L), f32)

    st = {}
    def fwd_chunk(a, shT, first, Dv=None):
        r0 = mo(a * C, C)
        kk = k_s[pl.ds(r0, C), :].astype(f32)
        for l in range(NL):
            kf_s[l, pl.ds(r0 + 8, C), :] = kk[:, l * L:(l + 1) * L]
        for l in range(NL):
            ls = slice(l * L, (l + 1) * L)
            Kf = jax.lax.dot_general(F_ref[...], ssm_s[ls, pl.ds(r0, C)], (((1,), (1,)), ((), ())),
                                     preferred_element_type=f32)
            if first:
                K_s[a, 0:C, ls] = Kf[0:C] + Dv[:, ls]
                K_s[a, C:, ls] = Kf[C:]
            else:
                K_s[a, :, ls] = Kf
            ks = kf_s[l, pl.ds(r0 + 8, C), :] * shT[0:1, ls]
            for j in range(1, 4):
                ks = ks + kf_s[l, pl.ds(r0 + 8 - j, C), :] * shT[j:j + 1, ls]
            kv = (ks * v_s[pl.ds(r0, C), ls].astype(f32)).astype(bf16)
            X_s[a, :, ls] = jnp.dot(F_ref[...], kv, preferred_element_type=f32)

    def t_mac(g, r0, l, Rr, jlo, jhi, init=None):
        a0 = GS * g
        init = (jlo == 0) if init is None else init

        def run():
            rre = pl.ds(mo(r0, Rr), Rr)
            rim = pl.ds(mo(r0 + C, Rr), Rr)
            ls = slice(l * L, (l + 1) * L)
            acc = [None] * GS
            kc = {}

            def getk(dl):
                if dl not in kc:
                    kr = K_s[dl, rre, ls]
                    ki = K_s[dl, rim, ls]
                    kc[dl] = (kr, ki, kr + ki)
                return kc[dl]

            for j in range(jlo, jhi):
                xr = X_s[j, rre, ls]
                xi = X_s[j, rim, ls]
                xs = xr + xi
                for t in range(GS):
                    dl = a0 + t - j
                    if dl < 0:
                        continue
                    kk = getk(dl)
                    terms = (kk[0] * xr, kk[1] * xi, kk[2] * xs)
                    acc[t] = terms if acc[t] is None else tuple(a + b for a, b in zip(acc[t], terms))
            for t in range(GS):
                if acc[t] is None:
                    continue
                P, Q, Rs = acc[t]
                yr, yi = P - Q, Rs - P - Q
                if not init:
                    yr = yr + Z_s[a0 + t, rre, ls]
                    yi = yi + Z_s[a0 + t, rim, ls]
                Z_s[a0 + t, rre, ls] = yr
                Z_s[a0 + t, rim, ls] = yi
        return run

    def mac_tasks(g, r_base, nrows, Rr, jb=None):
        out = []
        jend = GS * g + GS
        jb = jb or jend
        for dr in range(0, nrows, Rr):
            for l in range(NL):
                for j0 in range(0, jend, jb):
                    out.append(t_mac(g, r_base + dr, l, Rr, j0, min(j0 + jb, jend)))
        return out

    def mac_tasks_j(g, r_base, nrows, Rr, ranges, first_init):
        out = []
        for dr in range(0, nrows, Rr):
            for l in range(NL):
                for ii, (j0, j1) in enumerate(ranges):
                    out.append(t_mac(g, r_base + dr, l, Rr, j0, j1, first_init and ii == 0))
        return out

    def mac_loop(g):
        def body(i, _):
            interleave(mac_tasks(g, i * 16, 16, 16))
            return 0
        jax.lax.fori_loop(0, C // 16, body, 0)

    row = jax.lax.broadcasted_iota(jnp.int32, (C, L), 0)

    def t_inv(a, l, first):
        def run():
            ls = slice(l * L, (l + 1) * L)
            zr = Z_s[a, 0:C, ls]
            zi = Z_s[a, C:, ls]
            if not first:
                sgn = jnp.where((row & 1) == 0, 1.0, -1.0).astype(f32)
                zr = zr - sgn * Z_s[a - 1, C:, ls]
                zi = zi + sgn * Z_s[a - 1, 0:C, ls]
            w = jnp.concatenate([zr, zi], axis=0).astype(bf16)
            y_s[pl.ds(mo(a * C, C), C), ls] = jnp.dot(G_ref[...], w, preferred_element_type=f32)
        return run

    def inv_tasks(g):
        return [t_inv(g * GS + t, l, g == 0 and t == 0) for t in range(GS) for l in range(NL)]

    def t_post(r_dst, r_src, part):
        def run():
            rep = lambda i: jnp.concatenate([mod_s[i]] * (RB // 8), axis=0)
            if part in (0, 1):
                q = q_s[pl.ds(r_src, RB), :].astype(f32)
                m = jnp.mean(q, axis=-1, keepdims=True)
                xc = q - m
                r = jax.lax.rsqrt(jnp.mean(xc * xc, axis=-1, keepdims=True) + 1e-5)
                hg = (xc * r) * rep(0) + rep(1)
                x1 = hg * y_s[pl.ds(r_src, RB), :] + q
                x1_s[pl.ds(r_dst, RB), :] = x1
            if part == 2:
                x1 = x1_s[pl.ds(r_dst, RB), :]
            if part in (0, 2):
                m2 = jnp.mean(x1, axis=-1, keepdims=True)
                xc2 = x1 - m2
                r2 = jax.lax.rsqrt(jnp.mean(xc2 * xc2, axis=-1, keepdims=True) + 1e-5)
                h2_s[pl.ds(r_dst, RB), :] = ((xc2 * r2) * rep(2) + rep(3)).astype(bf16)
        return run

    def post_tasks(r_dst, r_src):
        out = []
        for t in range(BM // RB):
            a, b = mo(r_dst + t * RB, RB), mo(r_src + t * RB, RB)
            if CFG['pmode'] == 0:
                out.append(t_post(a, b, 0))
            else:
                out.append(t_post(a, b, 1))
                out.append(t_post(a, b, 2))
        return out

    def silu_c():
        cc = c_ref[...].astype(f32)
        return jnp.broadcast_to((cc * jax.nn.sigmoid(cc)).astype(bf16), (16, D))

    def ffn_iter(i, guard, others):
        ffn_iter_(i, guard, others)

    def ffn_iter_(i, guard, others):
        r0 = mo(i * BM, BM)
        fs = {'h2': h2_s[pl.ds(r0, BM), :]}
        tasks = []

        def guarded(fn):
            if guard is not None:
                fn()

        def t_gu(f):
            def run():
                wm = CFG['wmode']
                blk = lambda ff: range(ff * BF // WB, (ff + 1) * BF // WB)
                if wm == 0 and f > 0:
                    guarded(lambda: [(cp_wg(b).wait(), cp_wu(b).wait()) for b in blk(f)] and None)
                if wm == 2 and f > 0:
                    guarded(lambda: [(cp_wg(b).wait(), cp_wu(b).wait(), cp_wd(b).wait()) for b in blk(f)] and None)
                h2 = fs['h2']
                g = jnp.dot(h2, wg_s[:, f * BF:(f + 1) * BF], preferred_element_type=f32)
                u = jnp.dot(h2, wu_s[:, f * BF:(f + 1) * BF], preferred_element_type=f32)
                fs['act'] = (jnp.maximum(g, 0.0) * u).astype(bf16)
            return run

        def t_d(f):
            def run():
                wm = CFG['wmode']
                blk = lambda ff: range(ff * BF // WB, (ff + 1) * BF // WB)
                nf = Fd // BF
                if wm == 0 and f > 0:
                    guarded(lambda: [cp_wd(b).wait() for b in blk(f)] and None)
                if wm == 1:
                    def w():
                        if f == 0:
                            cp_q(1).wait()
                        for b in blk(f):
                            cp_wd(b).wait()
                        if f + 1 < nf and not (CFG.get('mid', True) and f + 2 == nf):
                            for b in blk(f + 1):
                                cp_wg(b).wait(); cp_wu(b).wait()
                    guarded(w)
                d = jnp.dot(fs['act'], wd_s[f * BF:(f + 1) * BF, :], preferred_element_type=f32)
                fs['acc'] = d if f == 0 else fs['acc'] + d
            return run

        for f in range(Fd // BF):
            tasks.append(t_gu(f))
            tasks.append(t_d(f))
        nxt = mo(jnp.minimum(r0 + BM, S - BM), BM)
        if guard is None:
            interleave(tasks, *others, post_tasks(r0 + BM, nxt))
        else:
            tasks[0]()
            if CFG.get('inv1late'):
                interleave(inv_tasks(1))
            if CFG.get('mid', True):
                pt = post_tasks(r0 + BM, nxt)
                interleave(tasks[1:-2], pt)
                st['late_fwd'](npre, npre + midc)
                for b in range((Fd - BF) // WB, nwb):
                    cp_wg(b).wait(); cp_wu(b).wait()
                interleave(tasks[-2:])
            else:
                interleave(tasks[1:], *others, post_tasks(r0 + BM, nxt))
            cp_wm(5).wait()
            mod_s[4] = jnp.dot(silu_c(), wm_s[:, 5 * D:6 * D], preferred_element_type=f32)[0:8]
        gbv = jnp.concatenate([mod_s[4]] * (BM // 8), axis=0)
        if CFG.get('osplit'):
            H = BM // 2
            for hh in range(2):
                rr = mo(r0 + hh * H, H)
                o_s[pl.ds(rr, H), :] = (x1_s[pl.ds(rr, H), :] + gbv[:H] * fs['acc'][hh * H:(hh + 1) * H]).astype(o_s.dtype)
                cp_oh(i, hh).start()
        else:
            o_s[pl.ds(r0, BM), :] = (x1_s[pl.ds(r0, BM), :] + gbv * fs['acc']).astype(o_s.dtype)
            cp_o(i).start()

    with scope("fwd0"):
        cp_k(0).wait(); cp_v(0).wait(); small[0].wait(); small[1].wait(); small[2].wait(); cp_ssm(0).wait()
        shT = shT_ref[...].astype(f32)
        Dv = D_ref[...].astype(f32).reshape(1, D)
        for t in range(CH):
            fwd_chunk(t, shT, t == 0, Dv)
    with scope("fwd"):
        def fbody(i, _):
            cp_k(i).wait(); cp_v(i).wait(); cp_ssm(i).wait()
            fwd_chunk(i, shT, False)
            return 0
        jax.lax.fori_loop(1, npre, fbody, 0)

    def late_fwd(lo, hi, extra=()):
        for cpy in late_copies(lo, hi):
            cpy.wait()
        sh = shT_ref[...].astype(f32)
        interleave([(lambda i=i: fwd_chunk(i, sh, False)) for i in range(lo, hi)], list(extra))
    st['late_fwd'] = late_fwd
    with scope("mac0"):
        mac_loop(0)
    with scope("inv0"):
        small[4].wait()
        interleave(inv_tasks(0))
    with scope("mac1"):
        mac_loop(1)
    with scope("mod"):
        small[3].wait()
        sc8 = silu_c()
        mods = [None] * 5
        for i in CFG.get('wm_order', (1, 0, 2, 4, 3)):
            cp_wm(i).wait()
            mods[i] = jnp.dot(sc8, wm_s[:, i * D:(i + 1) * D], preferred_element_type=f32)[0:8]
        sa, ca, ga, sb, cb = mods
        mod_s[0] = (1.0 + ca) * ga
        mod_s[1] = sa * ga
        mod_s[2] = 1.0 + cb
        mod_s[3] = sb
    with scope("inv1_post0"):
        cp_q(0).wait()
        interleave([] if CFG.get('inv1late') else inv_tasks(1), post_tasks(0, 0))
    with scope("wW"):
        for b in range(BF // WB):
            cp_wg(b).wait(); cp_wu(b).wait()
    with scope("P0"):
        def bodyP0(i, _):
            ffn_iter(i, True, [])
            return 0
        if CFG.get('p0loop'):
            jax.lax.fori_loop(0, 1, bodyP0, 0)
        else:
            bodyP0(0, 0)
    if npre + midc < 12:
        with scope("fwd2"):
            late_fwd(npre + midc, 12)
    with scope("A1"):
        cp_q(2).wait(); cp_q(3).wait()

        def bodyA1(i, _):
            extra = [mac_tasks_j(3, (i - 1) * 64, 64, 8, CFG['early3'], True)] if CFG.get('early3') else []
            ffn_iter(i, None, [mac_tasks(2, (i - 1) * 64, 64, 8, CFG['jb2'])] + extra)
            return 0
        jax.lax.fori_loop(1, 3, bodyA1, 0)
    if CFG.get('fuse23', True):
        with scope("inv2fwd3"):
            late_fwd(12, n, inv_tasks(2))
            for i in range(4, nq):
                cp_q(i).wait()
    else:
        with scope("inv2"):
            interleave(inv_tasks(2))
        with scope("fwd3"):
            late_fwd(12, n)
            for i in range(4, nq):
                cp_q(i).wait()
    with scope("A2"):
        def bodyA2(i, _):
            if CFG.get('early3'):
                ffn_iter(i, None, [mac_tasks_j(3, (i - 3) * 64, 64, 8, CFG['late3'], False)])
            else:
                ffn_iter(i, None, [mac_tasks(3, (i - 3) * 64, 64, 8, CFG['jb3'])])
            return 0
        jax.lax.fori_loop(3, 5, bodyA2, 0)
    with scope("inv3"):
        interleave(inv_tasks(3))
    with scope("B"):
        def bodyB(i, _):
            ffn_iter(i, None, [])
            return 0
        jax.lax.fori_loop(5, nq, bodyB, 0)
    with scope("drain"):
        for i in range(nq):
            if CFG.get('osplit'):
                cp_oh(i, 0).wait(); cp_oh(i, 1).wait()
            else:
                cp_o(i).wait()


@jax.jit
def pallas_adaLN_cond__ssm_conv_h3__glu_gated_reglu__prompt_kernel(A_q, A_k, A_v, A_shift_k, A_ssm_k, A_ssm_D, B_x, B_W_gate, B_W_up, B_W_down, c, w_mod):
    _, S, D = A_q.shape
    Fd = B_W_gate.shape[1]
    n = S // C
    BM = CFG['BM']
    nwb = Fd // CFG['WB']
    nsc = n // CFG['CH']
    any_ = pl.BlockSpec(memory_space=pl.ANY)
    V = pltpu.VMEM
    dma = pltpu.SemaphoreType.DMA
    out = pl.pallas_call(
        kernel,
        out_shape=jax.ShapeDtypeStruct((S, D), A_q.dtype),
        in_specs=[any_] * 13,
        out_specs=any_,
        scratch_shapes=[V((4, D), bf16), V((D,), bf16), V((1, D), bf16), V((2 * C, C), bf16), V((C, 2 * C), bf16),
                        V((S, D), bf16), V((S, D), bf16), V((S, D), bf16), V((D, S), bf16),
                        V((D, Fd), bf16), V((D, Fd), bf16), V((Fd, D), bf16), V((D, 6 * D), bf16),
                        V((D // L, S + 8, L), f32), V((n, 2 * C, D), f32), V((n, 2 * C, D), f32),
                        V((n, 2 * C, D), f32), V((S, D), f32), V((S + BM, D), f32),
                        V((S + BM, D), bf16), V((S, D), bf16),
                        V((5, 8, D), f32),
                        dma((5 + 3 * nsc + 6 + 3 * nwb + 3 * (S // BM),))],
        compiler_params=pltpu.CompilerParams(vmem_limit_bytes=120 * 1024 * 1024, flags=CFG.get("flags") or None),
    )(A_q[0], A_k[0], A_v[0], A_shift_k.T, A_ssm_k, A_ssm_D, B_W_gate, B_W_up, B_W_down, c, w_mod,
      jnp.asarray(_F), jnp.asarray(_G))
    return out[None]
```

```python
import numpy as np
import ml_dtypes
import jax
import jax.numpy as jnp
import jax.experimental.pallas as pl
import jax.experimental.pallas.tpu as pltpu

f32 = jnp.float32
bf16 = jnp.bfloat16

C = 128
L = 128
GS = 4
BM = 256
BF = 512
RB = 16
EPS = 1e-5


def _dft_mats():
    n = np.arange(C)[None, :].astype(np.float64)
    k = np.arange(C)[:, None].astype(np.float64)
    th = np.pi * (2 * k + 1) * n / (2 * C)
    fwd = np.concatenate([np.cos(th), -np.sin(th)], axis=0)
    inv = np.concatenate([np.cos(th).T, -np.sin(th).T], axis=1) / C
    cast = lambda a: a.astype(np.float32).astype(ml_dtypes.bfloat16)
    return cast(fwd), cast(inv)


_FWD, _INV = _dft_mats()


def _emit(*lists):
    items = []
    for li, tasks in enumerate(lists):
        for i, t in enumerate(tasks):
            items.append(((i + 0.5) / len(tasks), li, i, t))
    items.sort(key=lambda x: x[:3])
    for it in items:
        it[3]()


def _kernel(q_hbm, k_hbm, v_hbm, shT_hbm, ssm_hbm, D_hbm, wg_hbm, wu_hbm, wd_hbm, c_hbm, wm_hbm, F_hbm, G_hbm,
            o_hbm,
            shT_s, D_s, c_s, F_s, G_s, q_s, k_s, v_s, ssm_s, wg_s, wu_s, wd_s, wm_s,
            kf_s, X_s, K_s, Z_s, y_s, x1_s, h2_s, o_s, mod_s, sems):
    S, D = k_s.shape
    Fd = wd_s.shape[0]
    n = S // C
    NL = D // L
    nf = Fd // BF
    nq = S // BM
    half = BM // 2
    assert n == 4 * GS and nq == 8 and nf == 3 and BM == 2 * C

    off, tot = {}, 0
    for name, cnt in (('small', 5), ('k', n), ('v', n), ('ssm', n), ('q', nq), ('wm', 6), ('wg', nf), ('wu', nf),
                      ('wd', nf), ('o0', nq), ('o1', nq)):
        off[name] = tot
        tot += cnt
    sem = lambda name, i: sems.at[off[name] + i]
    mo = lambda r, m: r if isinstance(r, int) else pl.multiple_of(r, m)
    copy = pltpu.make_async_copy

    def cp_conv(a, cnt):
        rs = pl.ds(mo(a * C, C), cnt * C)
        return [copy(k_hbm.at[rs, :], k_s.at[rs, :], sem('k', a)),
                copy(v_hbm.at[rs, :], v_s.at[rs, :], sem('v', a)),
                copy(ssm_hbm.at[:, rs], ssm_s.at[:, rs], sem('ssm', a))]

    def cp_q(i):
        rs = pl.ds(i * BM, BM)
        return copy(q_hbm.at[rs, :], q_s.at[rs, :], sem('q', i))

    def cp_wm(i):
        cs = pl.ds(i * D, D)
        return copy(wm_hbm.at[:, cs], wm_s.at[:, cs], sem('wm', i))

    def cp_wg(i):
        cs = pl.ds(i * BF, BF)
        return copy(wg_hbm.at[:, cs], wg_s.at[:, cs], sem('wg', i))

    def cp_wu(i):
        cs = pl.ds(i * BF, BF)
        return copy(wu_hbm.at[:, cs], wu_s.at[:, cs], sem('wu', i))

    def cp_wd(i):
        rs = pl.ds(i * BF, BF)
        return copy(wd_hbm.at[rs, :], wd_s.at[rs, :], sem('wd', i))

    def cp_o(i, h):
        rs = pl.ds(mo(i * BM + h * half, half), half)
        return copy(o_s.at[rs, :], o_hbm.at[rs, :], sem('o1' if h else 'o0', i))

    cp_F, cp_sh, cp_D, cp_c, cp_G = [copy(a, b, sem('small', i)) for i, (a, b) in enumerate(
        ((F_hbm, F_s), (shT_hbm, shT_s), (D_hbm, D_s), (c_hbm, c_s), (G_hbm, G_s)))]
    wm_early = (1, 0, 2, 4, 3)

    def start(copies):
        for cp in copies:
            cp.start()

    def wait(copies):
        for cp in copies:
            cp.wait()

    k0, v0, ssm0 = cp_conv(0, 1)
    start([k0, v0, cp_F, cp_sh, cp_D, ssm0, cp_c, cp_G])
    for a in range(1, 8):
        start(cp_conv(a, 1))
    start([cp_wm(i) for i in wm_early])
    start([cp_q(0), cp_wg(0), cp_wu(0), cp_q(1), cp_wd(0), cp_wg(1), cp_wu(1), cp_wd(1)])
    start(cp_conv(8, 4))
    start([cp_wg(2), cp_wu(2), cp_wd(2), cp_wm(5), cp_q(2), cp_q(3)])
    start(cp_conv(12, 4))
    start([cp_q(i) for i in range(4, nq)])

    for l in range(NL):
        kf_s[l, 0:8, :] = jnp.zeros((8, L), f32)

    def fwd_chunk(a, shT, Dv=None):
        r0 = mo(a * C, C)
        kk = k_s[pl.ds(r0, C), :].astype(f32)
        for l in range(NL):
            kf_s[l, pl.ds(r0 + 8, C), :] = kk[:, l * L:(l + 1) * L]
        for l in range(NL):
            ls = slice(l * L, (l + 1) * L)
            Kf = jax.lax.dot_general(F_s[...], ssm_s[ls, pl.ds(r0, C)], (((1,), (1,)), ((), ())),
                                     preferred_element_type=f32)
            kre, kim = Kf[0:C], Kf[C:]
            if Dv is not None:
                kre = kre + Dv[:, ls]
            K_s[a, 0:C, ls] = kre
            K_s[a, C:, ls] = kim
            ks = kf_s[l, pl.ds(r0 + 8, C), :] * shT[0:1, ls]
            for j in range(1, 4):
                ks = ks + kf_s[l, pl.ds(r0 + 8 - j, C), :] * shT[j:j + 1, ls]
            kv = (ks * v_s[pl.ds(r0, C), ls].astype(f32)).astype(bf16)
            X_s[a, :, ls] = jnp.dot(F_s[...], kv, preferred_element_type=f32)

    def late_fwd(a0, extra=()):
        wait(cp_conv(a0, GS))
        shT = shT_s[...].astype(f32)
        _emit([(lambda a=a: fwd_chunk(a, shT)) for a in range(a0, a0 + GS)], list(extra))

    def mac_task(g, r0, l, rows, jlo, jhi, init):
        a0 = GS * g

        def run():
            rre = pl.ds(mo(r0, rows), rows)
            rim = pl.ds(mo(r0 + C, rows), rows)
            ls = slice(l * L, (l + 1) * L)
            acc = [None] * GS
            kc = {}

            def getk(d):
                if d not in kc:
                    kr = K_s[d, rre, ls]
                    ki = K_s[d, rim, ls]
                    kc[d] = (kr, ki, kr + ki)
                return kc[d]

            for j in range(jlo, jhi):
                xr = X_s[j, rre, ls]
                xi = X_s[j, rim, ls]
                xs = xr + xi
                for t in range(GS):
                    d = a0 + t - j
                    if d < 0:
                        continue
                    kr, ki, ks = getk(d)
                    terms = (kr * xr, ki * xi, ks * xs)
                    acc[t] = terms if acc[t] is None else tuple(p + s for p, s in zip(acc[t], terms))
            for t in range(GS):
                if acc[t] is None:
                    continue
                P, Q, R = acc[t]
                yr, yi = P - Q, R - P - Q
                if not init:
                    yr = yr + Z_s[a0 + t, rre, ls]
                    yi = yi + Z_s[a0 + t, rim, ls]
                Z_s[a0 + t, rre, ls] = yr
                Z_s[a0 + t, rim, ls] = yi
        return run

    def mac_tasks(g, r_base, nrows, rows, ranges, init):
        return [mac_task(g, r_base + dr, l, rows, j0, j1, init and i == 0)
                for dr in range(0, nrows, rows) for l in range(NL) for i, (j0, j1) in enumerate(ranges)]

    def mac_group(g):
        def body(i, _):
            _emit(mac_tasks(g, i * 16, 16, 16, [(0, GS * g + GS)], True))
            return 0
        jax.lax.fori_loop(0, C // 16, body, 0)

    row = jax.lax.broadcasted_iota(jnp.int32, (C, L), 0)

    def inv_task(a, l):
        def run():
            ls = slice(l * L, (l + 1) * L)
            zr = Z_s[a, 0:C, ls]
            zi = Z_s[a, C:, ls]
            if a > 0:
                sgn = jnp.where((row & 1) == 0, 1.0, -1.0).astype(f32)
                zr = zr - sgn * Z_s[a - 1, C:, ls]
                zi = zi + sgn * Z_s[a - 1, 0:C, ls]
            w = jnp.concatenate([zr, zi], axis=0).astype(bf16)
            y_s[a * C:(a + 1) * C, ls] = jnp.dot(G_s[...], w, preferred_element_type=f32)
        return run

    def inv_tasks(g):
        return [inv_task(g * GS + t, l) for t in range(GS) for l in range(NL)]

    def rep(i, rows):
        return jnp.concatenate([mod_s[i]] * (rows // 8), axis=0)

    def x1_task(r_dst, r_src):
        def run():
            q = q_s[pl.ds(r_src, RB), :].astype(f32)
            xc = q - jnp.mean(q, axis=-1, keepdims=True)
            r = jax.lax.rsqrt(jnp.mean(xc * xc, axis=-1, keepdims=True) + EPS)
            hg = (xc * r) * rep(0, RB) + rep(1, RB)
            x1_s[pl.ds(r_dst, RB), :] = hg * y_s[pl.ds(r_src, RB), :] + q
        return run

    def h2_task(r_dst):
        def run():
            x1 = x1_s[pl.ds(r_dst, RB), :]
            xc = x1 - jnp.mean(x1, axis=-1, keepdims=True)
            r = jax.lax.rsqrt(jnp.mean(xc * xc, axis=-1, keepdims=True) + EPS)
            h2_s[pl.ds(r_dst, RB), :] = ((xc * r) * rep(2, RB) + rep(3, RB)).astype(bf16)
        return run

    def norm_tasks(r_dst, r_src):
        out = []
        for t in range(BM // RB):
            a, b = mo(r_dst + t * RB, RB), mo(r_src + t * RB, RB)
            out += [x1_task(a, b), h2_task(a)]
        return out

    def silu_c():
        cc = c_s[...].astype(f32)
        return jnp.broadcast_to((cc * jax.nn.sigmoid(cc)).astype(bf16), (16, D))

    def mod_piece(sc, i):
        return jnp.dot(sc, wm_s[:, i * D:(i + 1) * D], preferred_element_type=f32)[0:8]

    def ffn_tasks(r0):
        st = {'h2': h2_s[pl.ds(r0, BM), :]}

        def gate_up(f):
            def run():
                cs = slice(f * BF, (f + 1) * BF)
                g = jnp.dot(st['h2'], wg_s[:, cs], preferred_element_type=f32)
                u = jnp.dot(st['h2'], wu_s[:, cs], preferred_element_type=f32)
                st['act'] = (jnp.maximum(g, 0.0) * u).astype(bf16)
            return run

        def down(f):
            def run():
                d = jnp.dot(st['act'], wd_s[f * BF:(f + 1) * BF, :], preferred_element_type=f32)
                st['acc'] = d if f == 0 else st['acc'] + d
            return run

        return st, [t for f in range(nf) for t in (gate_up(f), down(f))]

    def write_out(i, r0, acc):
        gb = rep(4, half)
        for h in range(2):
            rs = pl.ds(mo(r0 + h * half, half), half)
            o_s[rs, :] = (x1_s[rs, :] + gb * acc[h * half:(h + 1) * half]).astype(o_s.dtype)
            cp_o(i, h).start()

    def ffn_step(i, *others):
        r0 = mo(i * BM, BM)
        st, tasks = ffn_tasks(r0)
        nxt = mo(jnp.minimum(r0 + BM, S - BM), BM)
        _emit(tasks, *others, norm_tasks(r0 + BM, nxt))
        write_out(i, r0, st['acc'])

    wait([k0, v0, cp_F, cp_sh, cp_D, ssm0])
    shT = shT_s[...].astype(f32)
    fwd_chunk(0, shT, D_s[...].astype(f32).reshape(1, D))

    def fwd_body(a, _):
        wait(cp_conv(a, 1))
        fwd_chunk(a, shT)
        return 0
    jax.lax.fori_loop(1, 8, fwd_body, 0)

    mac_group(0)
    cp_G.wait()
    _emit(inv_tasks(0))
    mac_group(1)

    cp_c.wait()
    sc = silu_c()
    m = [None] * 5
    for i in wm_early:
        cp_wm(i).wait()
        m[i] = mod_piece(sc, i)
    sa, ca, ga, sb, cb = m
    mod_s[0] = (1.0 + ca) * ga
    mod_s[1] = sa * ga
    mod_s[2] = 1.0 + cb
    mod_s[3] = sb

    cp_q(0).wait()
    _emit(norm_tasks(0, 0))

    wait([cp_wg(0), cp_wu(0)])
    st, tasks = ffn_tasks(0)
    gu0, d0, gu1, d1, gu2, d2 = tasks
    gu0()
    _emit(inv_tasks(1))

    def waited(copies, task):
        def run():
            wait(copies)
            task()
        return run
    _emit([waited([cp_q(1), cp_wd(0), cp_wg(1), cp_wu(1)], d0), gu1, waited([cp_wd(1)], d1)], norm_tasks(BM, BM))
    late_fwd(8)
    wait([cp_wg(2), cp_wu(2)])
    gu2()
    wait([cp_wd(2)])
    d2()
    cp_wm(5).wait()
    mod_s[4] = mod_piece(silu_c(), 5)
    write_out(0, 0, st['acc'])

    wait([cp_q(2), cp_q(3)])

    def step_a1(i, _):
        rb = (i - 1) * (C // 2)
        ffn_step(i, mac_tasks(2, rb, C // 2, 8, [(j, j + 2) for j in range(0, 12, 2)], True),
                 mac_tasks(3, rb, C // 2, 8, [(4, 6), (6, 8)], True))
        return 0
    jax.lax.fori_loop(1, 3, step_a1, 0)

    late_fwd(12, inv_tasks(2))
    wait([cp_q(i) for i in range(4, nq)])

    def step_a2(i, _):
        rb = (i - 3) * (C // 2)
        ffn_step(i, mac_tasks(3, rb, C // 2, 8, [(0, 2), (2, 4), (8, 10), (10, 12), (12, 14), (14, 16)], False))
        return 0
    jax.lax.fori_loop(3, 5, step_a2, 0)

    _emit(inv_tasks(3))

    def step_b(i, _):
        ffn_step(i)
        return 0
    jax.lax.fori_loop(5, nq, step_b, 0)

    wait([cp_o(i, h) for i in range(nq) for h in range(2)])


@jax.jit
def pallas_adaLN_cond__ssm_conv_h3__glu_gated_reglu__prompt_kernel(A_q, A_k, A_v, A_shift_k, A_ssm_k, A_ssm_D, B_x, B_W_gate, B_W_up, B_W_down, c, w_mod):
    del B_x
    _, S, D = A_q.shape
    Fd = B_W_gate.shape[1]
    n = S // C
    V = pltpu.VMEM
    hbm = pl.BlockSpec(memory_space=pl.ANY)
    n_sems = 5 + 3 * n + 6 + 3 * (Fd // BF) + 3 * (S // BM)
    out = pl.pallas_call(
        _kernel,
        out_shape=jax.ShapeDtypeStruct((S, D), A_q.dtype),
        in_specs=[hbm] * 13,
        out_specs=hbm,
        scratch_shapes=[
            V((4, D), bf16), V((D,), bf16), V((1, D), bf16), V((2 * C, C), bf16), V((C, 2 * C), bf16),
            V((S, D), bf16), V((S, D), bf16), V((S, D), bf16), V((D, S), bf16),
            V((D, Fd), bf16), V((D, Fd), bf16), V((Fd, D), bf16), V((D, 6 * D), bf16),
            V((D // L, S + 8, L), f32),
            V((n, 2 * C, D), f32), V((n, 2 * C, D), f32), V((n, 2 * C, D), f32),
            V((S, D), f32),
            V((S + BM, D), f32), V((S + BM, D), bf16),
            V((S, D), bf16),
            V((5, 8, D), f32),
            pltpu.SemaphoreType.DMA((n_sems,)),
        ],
        compiler_params=pltpu.CompilerParams(vmem_limit_bytes=120 * 1024 * 1024),
    )(A_q[0], A_k[0], A_v[0], A_shift_k.T, A_ssm_k, A_ssm_D, B_W_gate, B_W_up, B_W_down, c, w_mod,
      jnp.asarray(_FWD), jnp.asarray(_INV))
    return out[None]
```

```python
import numpy as np
import ml_dtypes
import jax
import jax.numpy as jnp
import jax.experimental.pallas as pl
import jax.experimental.pallas.tpu as pltpu

f32 = jnp.float32
bf16 = jnp.bfloat16

C = 128
L = 128
GS = 4
BM = 256
BF = 512
RB = 16
EPS = 1e-5


def _dft_mats():
    n = np.arange(C)[None, :].astype(np.float64)
    k = np.arange(C)[:, None].astype(np.float64)
    th = np.pi * (2 * k + 1) * n / (2 * C)
    fwd = np.concatenate([np.cos(th), -np.sin(th)], axis=0)
    inv = np.concatenate([np.cos(th).T, -np.sin(th).T], axis=1) / C
    cast = lambda a: a.astype(np.float32).astype(ml_dtypes.bfloat16)
    return cast(fwd), cast(inv)


_FWD, _INV = _dft_mats()


def _emit(*lists):
    items = []
    for li, tasks in enumerate(lists):
        for i, t in enumerate(tasks):
            items.append(((i + 0.5) / len(tasks), li, i, t))
    items.sort(key=lambda x: x[:3])
    for it in items:
        it[3]()


def _kernel(q_hbm, k_hbm, v_hbm, shT_hbm, ssm_hbm, D_hbm, wg_hbm, wu_hbm, wd_hbm, c_hbm, wm_hbm, F_hbm, G_hbm,
            o_hbm,
            shT_s, D_s, c_s, F_s, G_s, q_s, k_s, v_s, ssm_s, wg_s, wu_s, wd_s, wm_s,
            kf_s, X_s, K_s, Z_s, y_s, x1_s, h2_s, o_s, mod_s, sems):
    S, D = k_s.shape
    Fd = wd_s.shape[0]
    n = S // C
    NL = D // L
    nf = Fd // BF
    nq = S // BM
    half = BM // 2
    assert n == 4 * GS and nq == 8 and nf == 3 and BM == 2 * C

    off, tot = {}, 0
    for name, cnt in (('small', 5), ('k', n), ('v', n), ('ssm', n), ('q', nq), ('wm', 6), ('wg', nf), ('wu', nf),
                      ('wd', nf), ('o0', nq), ('o1', nq)):
        off[name] = tot
        tot += cnt
    sem = lambda name, i: sems.at[off[name] + i]
    mo = lambda r, m: r if isinstance(r, int) else pl.multiple_of(r, m)
    copy = pltpu.make_async_copy

    def cp_conv(a, cnt):
        rs = pl.ds(mo(a * C, C), cnt * C)
        return [copy(k_hbm.at[rs, :], k_s.at[rs, :], sem('k', a)),
                copy(v_hbm.at[rs, :], v_s.at[rs, :], sem('v', a)),
                copy(ssm_hbm.at[:, rs], ssm_s.at[:, rs], sem('ssm', a))]

    def cp_q(i):
        rs = pl.ds(i * BM, BM)
        return copy(q_hbm.at[rs, :], q_s.at[rs, :], sem('q', i))

    def cp_wm(i):
        cs = pl.ds(i * D, D)
        return copy(wm_hbm.at[:, cs], wm_s.at[:, cs], sem('wm', i))

    def cp_wg(i):
        cs = pl.ds(i * BF, BF)
        return copy(wg_hbm.at[:, cs], wg_s.at[:, cs], sem('wg', i))

    def cp_wu(i):
        cs = pl.ds(i * BF, BF)
        return copy(wu_hbm.at[:, cs], wu_s.at[:, cs], sem('wu', i))

    def cp_wd(i):
        rs = pl.ds(i * BF, BF)
        return copy(wd_hbm.at[rs, :], wd_s.at[rs, :], sem('wd', i))

    def cp_o(i, h):
        rs = pl.ds(mo(i * BM + h * half, half), half)
        return copy(o_s.at[rs, :], o_hbm.at[rs, :], sem('o1' if h else 'o0', i))

    cp_F, cp_sh, cp_D, cp_c, cp_G = [copy(a, b, sem('small', i)) for i, (a, b) in enumerate(
        ((F_hbm, F_s), (shT_hbm, shT_s), (D_hbm, D_s), (c_hbm, c_s), (G_hbm, G_s)))]
    wm_early = (1, 0, 2, 4, 3)

    def start(copies):
        for cp in copies:
            cp.start()

    def wait(copies):
        for cp in copies:
            cp.wait()

    k0, v0, ssm0 = cp_conv(0, 1)
    start([k0, v0, cp_F, cp_sh, cp_D, ssm0, cp_c, cp_G])
    for a in range(1, 8):
        start(cp_conv(a, 1))
    start([cp_wm(i) for i in wm_early])
    start([cp_q(0), cp_wg(0), cp_wu(0), cp_q(1), cp_wd(0), cp_wg(1), cp_wu(1), cp_wd(1)])
    start(cp_conv(8, 4))
    start([cp_wg(2), cp_wu(2), cp_wd(2), cp_wm(5), cp_q(2), cp_q(3)])
    start(cp_conv(12, 4))
    start([cp_q(i) for i in range(4, nq)])

    for l in range(NL):
        kf_s[l, 0:8, :] = jnp.zeros((8, L), f32)

    def fwd_chunk(a, shT, Dv=None):
        r0 = mo(a * C, C)
        kk = k_s[pl.ds(r0, C), :].astype(f32)
        for l in range(NL):
            kf_s[l, pl.ds(r0 + 8, C), :] = kk[:, l * L:(l + 1) * L]
        for l in range(NL):
            ls = slice(l * L, (l + 1) * L)
            Kf = jax.lax.dot_general(F_s[...], ssm_s[ls, pl.ds(r0, C)], (((1,), (1,)), ((), ())),
                                     preferred_element_type=f32)
            kre, kim = Kf[0:C], Kf[C:]
            if Dv is not None:
                kre = kre + Dv[:, ls]
            K_s[a, 0:C, ls] = kre
            K_s[a, C:, ls] = kim
            ks = kf_s[l, pl.ds(r0 + 8, C), :] * shT[0:1, ls]
            for j in range(1, 4):
                ks = ks + kf_s[l, pl.ds(r0 + 8 - j, C), :] * shT[j:j + 1, ls]
            kv = (ks * v_s[pl.ds(r0, C), ls].astype(f32)).astype(bf16)
            X_s[a, :, ls] = jnp.dot(F_s[...], kv, preferred_element_type=f32)

    def late_fwd(a0, extra=()):
        wait(cp_conv(a0, GS))
        shT = shT_s[...].astype(f32)
        _emit([(lambda a=a: fwd_chunk(a, shT)) for a in range(a0, a0 + GS)], list(extra))

    def mac_task(g, r0, l, rows, jlo, jhi, init):
        a0 = GS * g

        def run():
            rre = pl.ds(mo(r0, rows), rows)
            rim = pl.ds(mo(r0 + C, rows), rows)
            ls = slice(l * L, (l + 1) * L)
            acc = [None] * GS
            kc = {}

            def getk(d):
                if d not in kc:
                    kr = K_s[d, rre, ls]
                    ki = K_s[d, rim, ls]
                    kc[d] = (kr, ki, kr + ki)
                return kc[d]

            for j in range(jlo, jhi):
                xr = X_s[j, rre, ls]
                xi = X_s[j, rim, ls]
                xs = xr + xi
                for t in range(GS):
                    d = a0 + t - j
                    if d < 0:
                        continue
                    kr, ki, ks = getk(d)
                    terms = (kr * xr, ki * xi, ks * xs)
                    acc[t] = terms if acc[t] is None else tuple(p + s for p, s in zip(acc[t], terms))
            for t in range(GS):
                if acc[t] is None:
                    continue
                P, Q, R = acc[t]
                yr, yi = P - Q, R - P - Q
                if not init:
                    yr = yr + Z_s[a0 + t, rre, ls]
                    yi = yi + Z_s[a0 + t, rim, ls]
                Z_s[a0 + t, rre, ls] = yr
                Z_s[a0 + t, rim, ls] = yi
        return run

    def mac_tasks(g, r_base, nrows, rows, ranges, init):
        return [mac_task(g, r_base + dr, l, rows, j0, j1, init and i == 0)
                for dr in range(0, nrows, rows) for l in range(NL) for i, (j0, j1) in enumerate(ranges)]

    def mac_group(g):
        def body(i, _):
            _emit(mac_tasks(g, i * 16, 16, 16, [(0, GS * g + GS)], True))
            return 0
        jax.lax.fori_loop(0, C // 16, body, 0)

    row = jax.lax.broadcasted_iota(jnp.int32, (C, L), 0)

    def inv_task(a, l):
        def run():
            ls = slice(l * L, (l + 1) * L)
            zr = Z_s[a, 0:C, ls]
            zi = Z_s[a, C:, ls]
            if a > 0:
                sgn = jnp.where((row & 1) == 0, 1.0, -1.0).astype(f32)
                zr = zr - sgn * Z_s[a - 1, C:, ls]
                zi = zi + sgn * Z_s[a - 1, 0:C, ls]
            w = jnp.concatenate([zr, zi], axis=0).astype(bf16)
            y_s[a * C:(a + 1) * C, ls] = jnp.dot(G_s[...], w, preferred_element_type=f32)
        return run

    def inv_tasks(g):
        return [inv_task(g * GS + t, l) for t in range(GS) for l in range(NL)]

    def rep(i, rows):
        return jnp.concatenate([mod_s[i]] * (rows // 8), axis=0)

    def x1_task(r_dst, r_src):
        def run():
            q = q_s[pl.ds(r_src, RB), :].astype(f32)
            xc = q - jnp.mean(q, axis=-1, keepdims=True)
            r = jax.lax.rsqrt(jnp.mean(xc * xc, axis=-1, keepdims=True) + EPS)
            hg = (xc * r) * rep(0, RB) + rep(1, RB)
            x1_s[pl.ds(r_dst, RB), :] = hg * y_s[pl.ds(r_src, RB), :] + q
        return run

    def h2_task(r_dst, r_x1):
        def run():
            x1 = x1_s[pl.ds(r_x1, RB), :]
            xc = x1 - jnp.mean(x1, axis=-1, keepdims=True)
            r = jax.lax.rsqrt(jnp.mean(xc * xc, axis=-1, keepdims=True) + EPS)
            h2_s[pl.ds(r_dst, RB), :] = ((xc * r) * rep(2, RB) + rep(3, RB)).astype(bf16)
        return run

    def norm_tasks(r_dst, r_src, with_x1=True):
        out = []
        for t in range(BM // RB):
            a, b = mo(r_dst + t * RB, RB), mo(r_src + t * RB, RB)
            out += [x1_task(a, b), h2_task(a, a)] if with_x1 else [h2_task(a, b)]
        return out

    def silu_c():
        cc = c_s[...].astype(f32)
        return jnp.broadcast_to((cc * jax.nn.sigmoid(cc)).astype(bf16), (16, D))

    def mod_piece(sc, i):
        return jnp.dot(sc, wm_s[:, i * D:(i + 1) * D], preferred_element_type=f32)[0:8]

    def ffn_tasks(r0):
        st = {'h2': h2_s[pl.ds(r0, BM), :]}

        def gate_up(f):
            def run():
                cs = slice(f * BF, (f + 1) * BF)
                g = jnp.dot(st['h2'], wg_s[:, cs], preferred_element_type=f32)
                u = jnp.dot(st['h2'], wu_s[:, cs], preferred_element_type=f32)
                st['act'] = (jnp.maximum(g, 0.0) * u).astype(bf16)
            return run

        def down(f):
            def run():
                d = jnp.dot(st['act'], wd_s[f * BF:(f + 1) * BF, :], preferred_element_type=f32)
                st['acc'] = d if f == 0 else st['acc'] + d
            return run

        return st, [t for f in range(nf) for t in (gate_up(f), down(f))]

    def write_out(i, r0, acc):
        gb = rep(4, half)
        for h in range(2):
            rs = pl.ds(mo(r0 + h * half, half), half)
            o_s[rs, :] = (x1_s[rs, :] + gb * acc[h * half:(h + 1) * half]).astype(o_s.dtype)
            cp_o(i, h).start()

    def ffn_step(i, *others, with_x1=True):
        r0 = mo(i * BM, BM)
        st, tasks = ffn_tasks(r0)
        nxt = mo(jnp.minimum(r0 + BM, S - BM), BM)
        _emit(tasks, *others, norm_tasks(r0 + BM, nxt, with_x1))
        write_out(i, r0, st['acc'])

    wait([k0, v0, cp_F, cp_sh, cp_D, ssm0])
    shT = shT_s[...].astype(f32)
    fwd_chunk(0, shT, D_s[...].astype(f32).reshape(1, D))

    def fwd_body(a, _):
        wait(cp_conv(a, 1))
        fwd_chunk(a, shT)
        return 0
    jax.lax.fori_loop(1, 8, fwd_body, 0)

    mac_group(0)
    cp_G.wait()
    _emit(inv_tasks(0))
    mac_group(1)

    cp_c.wait()
    sc = silu_c()
    m = [None] * 5
    for i in wm_early:
        cp_wm(i).wait()
        m[i] = mod_piece(sc, i)
    sa, ca, ga, sb, cb = m
    mod_s[0] = (1.0 + ca) * ga
    mod_s[1] = sa * ga
    mod_s[2] = 1.0 + cb
    mod_s[3] = sb

    cp_q(0).wait()
    _emit(norm_tasks(0, 0))

    wait([cp_wg(0), cp_wu(0)])
    st, tasks = ffn_tasks(0)
    gu0, d0, gu1, d1, gu2, d2 = tasks
    gu0()
    _emit(inv_tasks(1))

    def waited(copies, task):
        def run():
            wait(copies)
            task()
        return run
    _emit([waited([cp_q(1), cp_wd(0), cp_wg(1), cp_wu(1)], d0), gu1, waited([cp_wd(1)], d1)], norm_tasks(BM, BM))
    late_fwd(8)
    wait([cp_wg(2), cp_wu(2)])
    gu2()
    wait([cp_wd(2), cp_wm(5)])
    mod_s[4] = mod_piece(silu_c(), 5)
    d2()
    write_out(0, 0, st['acc'])

    wait([cp_q(2), cp_q(3)])

    def step_a1(i, _):
        rb = (i - 1) * (C // 2)
        ffn_step(i, mac_tasks(2, rb, C // 2, 8, [(j, j + 2) for j in range(0, 12, 2)], True),
                 mac_tasks(3, rb, C // 2, 8, [(4, 6), (6, 8)], True))
        return 0
    jax.lax.fori_loop(1, 3, step_a1, 0)

    wait([cp_q(i) for i in range(4, nq)])
    chain = []
    for a in range(8, 12):
        chain += [inv_task(a, l) for l in range(NL)]
        chain += [x1_task(r, r) for r in range(a * C, (a + 1) * C, RB)]
    late_fwd(12, chain)

    def step_a2(i, _):
        rb = (i - 3) * (C // 2)
        ffn_step(i, mac_tasks(3, rb, C // 2, 8, [(0, 2), (2, 4), (8, 10), (10, 12), (12, 14), (14, 16)], False), with_x1=False)
        return 0
    jax.lax.fori_loop(3, 5, step_a2, 0)

    _emit(inv_tasks(3) + [x1_task(r, r) for r in range(12 * C, 16 * C, RB)])

    def step_b(i, _):
        ffn_step(i, with_x1=False)
        return 0
    jax.lax.fori_loop(5, nq, step_b, 0)

    wait([cp_o(i, h) for i in range(nq) for h in range(2)])


@jax.jit
def pallas_adaLN_cond__ssm_conv_h3__glu_gated_reglu__prompt_kernel(A_q, A_k, A_v, A_shift_k, A_ssm_k, A_ssm_D, B_x, B_W_gate, B_W_up, B_W_down, c, w_mod):
    del B_x
    _, S, D = A_q.shape
    Fd = B_W_gate.shape[1]
    n = S // C
    V = pltpu.VMEM
    hbm = pl.BlockSpec(memory_space=pl.ANY)
    n_sems = 5 + 3 * n + 6 + 3 * (Fd // BF) + 3 * (S // BM)
    out = pl.pallas_call(
        _kernel,
        out_shape=jax.ShapeDtypeStruct((S, D), A_q.dtype),
        in_specs=[hbm] * 13,
        out_specs=hbm,
        scratch_shapes=[
            V((4, D), bf16), V((D,), bf16), V((1, D), bf16), V((2 * C, C), bf16), V((C, 2 * C), bf16),
            V((S, D), bf16), V((S, D), bf16), V((S, D), bf16), V((D, S), bf16),
            V((D, Fd), bf16), V((D, Fd), bf16), V((Fd, D), bf16), V((D, 6 * D), bf16),
            V((D // L, S + 8, L), f32),
            V((n, 2 * C, D), f32), V((n, 2 * C, D), f32), V((n, 2 * C, D), f32),
            V((S, D), f32),
            V((S + BM, D), f32), V((S + BM, D), bf16),
            V((S, D), bf16),
            V((5, 8, D), f32),
            pltpu.SemaphoreType.DMA((n_sems,)),
        ],
        compiler_params=pltpu.CompilerParams(vmem_limit_bytes=120 * 1024 * 1024),
    )(A_q[0], A_k[0], A_v[0], A_shift_k.T, A_ssm_k, A_ssm_D, B_W_gate, B_W_up, B_W_down, c, w_mod,
      jnp.asarray(_FWD), jnp.asarray(_INV))
    return out[None]
```

```python
import numpy as np
import ml_dtypes
import jax
import jax.numpy as jnp
import jax.experimental.pallas as pl
import jax.experimental.pallas.tpu as pltpu

f32 = jnp.float32
bf16 = jnp.bfloat16

C = 128
L = 128
GS = 4
BM = 256
BF = 512
RB = 16
EPS = 1e-5


def _dft_mats():
    n = np.arange(C)[None, :].astype(np.float64)
    k = np.arange(C)[:, None].astype(np.float64)
    th = np.pi * (2 * k + 1) * n / (2 * C)
    fwd = np.concatenate([np.cos(th), -np.sin(th)], axis=0)
    inv = np.concatenate([np.cos(th).T, -np.sin(th).T], axis=1) / C
    cast = lambda a: a.astype(np.float32).astype(ml_dtypes.bfloat16)
    return cast(fwd), cast(inv)


_FWD, _INV = _dft_mats()


def _emit(*lists):
    items = []
    for li, tasks in enumerate(lists):
        for i, t in enumerate(tasks):
            items.append(((i + 0.5) / len(tasks), li, i, t))
    items.sort(key=lambda x: x[:3])
    for it in items:
        it[3]()


def _kernel(q_hbm, k_hbm, v_hbm, shT_hbm, ssm_hbm, D_hbm, wg_hbm, wu_hbm, wd_hbm, c_hbm, wm_hbm, F_hbm, G_hbm,
            o_hbm,
            shT_s, D_s, c_s, F_s, G_s, q_s, k_s, v_s, ssm_s, wg_s, wu_s, wd_s, wm_s,
            kf_s, X_s, K_s, Z_s, y_s, x1_s, h2_s, o_s, mod_s, sems):
    S, D = k_s.shape
    Fd = wd_s.shape[0]
    n = S // C
    NL = D // L
    nf = Fd // BF
    nq = S // BM
    half = BM // 2
    assert n == 4 * GS and nq == 8 and nf == 3 and BM == 2 * C

    off, tot = {}, 0
    for name, cnt in (('small', 5), ('k', n), ('v', n), ('ssm', n), ('q', nq), ('wm', 6), ('wg', nf), ('wu', nf),
                      ('wd', nf), ('o0', nq), ('o1', nq)):
        off[name] = tot
        tot += cnt
    sem = lambda name, i: sems.at[off[name] + i]
    mo = lambda r, m: r if isinstance(r, int) else pl.multiple_of(r, m)
    copy = pltpu.make_async_copy

    def cp_conv(a, cnt):
        rs = pl.ds(mo(a * C, C), cnt * C)
        return [copy(k_hbm.at[rs, :], k_s.at[rs, :], sem('k', a)),
                copy(v_hbm.at[rs, :], v_s.at[rs, :], sem('v', a)),
                copy(ssm_hbm.at[:, rs], ssm_s.at[:, rs], sem('ssm', a))]

    def cp_q(i):
        rs = pl.ds(i * BM, BM)
        return copy(q_hbm.at[rs, :], q_s.at[rs, :], sem('q', i))

    def cp_wm(i):
        cs = pl.ds(i * D, D)
        return copy(wm_hbm.at[:, cs], wm_s.at[:, cs], sem('wm', i))

    def cp_wg(i):
        cs = pl.ds(i * BF, BF)
        return copy(wg_hbm.at[:, cs], wg_s.at[:, cs], sem('wg', i))

    def cp_wu(i):
        cs = pl.ds(i * BF, BF)
        return copy(wu_hbm.at[:, cs], wu_s.at[:, cs], sem('wu', i))

    def cp_wd(i):
        rs = pl.ds(i * BF, BF)
        return copy(wd_hbm.at[rs, :], wd_s.at[rs, :], sem('wd', i))

    def cp_o(i, h):
        rs = pl.ds(mo(i * BM + h * half, half), half)
        return copy(o_s.at[rs, :], o_hbm.at[rs, :], sem('o1' if h else 'o0', i))

    cp_F, cp_sh, cp_D, cp_c, cp_G = [copy(a, b, sem('small', i)) for i, (a, b) in enumerate(
        ((F_hbm, F_s), (shT_hbm, shT_s), (D_hbm, D_s), (c_hbm, c_s), (G_hbm, G_s)))]
    wm_early = (1, 0, 2, 4, 3)

    def start(copies):
        for cp in copies:
            cp.start()

    def wait(copies):
        for cp in copies:
            cp.wait()

    k0, v0, ssm0 = cp_conv(0, 1)
    start([k0, v0, cp_F, cp_sh, cp_D, ssm0, cp_c, cp_G])
    for a in range(1, 8):
        start(cp_conv(a, 1))
    start([cp_wm(i) for i in wm_early])
    start([cp_q(0), cp_wg(0), cp_wu(0), cp_q(1), cp_wd(0), cp_wg(1), cp_wu(1), cp_wd(1)])
    start(cp_conv(8, 4))
    start([cp_wg(2), cp_wu(2), cp_wd(2), cp_wm(5), cp_q(2), cp_q(3)])
    start(cp_conv(12, 4))
    start([cp_q(i) for i in range(4, nq)])

    for l in range(NL):
        kf_s[l, 0:8, :] = jnp.zeros((8, L), f32)

    def fwd_chunk(a, shT, Dv=None):
        r0 = mo(a * C, C)
        kk = k_s[pl.ds(r0, C), :].astype(f32)
        for l in range(NL):
            kf_s[l, pl.ds(r0 + 8, C), :] = kk[:, l * L:(l + 1) * L]
        for l in range(NL):
            ls = slice(l * L, (l + 1) * L)
            Kf = jax.lax.dot_general(F_s[...], ssm_s[ls, pl.ds(r0, C)], (((1,), (1,)), ((), ())),
                                     preferred_element_type=f32)
            kre, kim = Kf[0:C], Kf[C:]
            if Dv is not None:
                kre = kre + Dv[:, ls]
            K_s[a, 0:C, ls] = kre
            K_s[a, C:, ls] = kim
            ks = kf_s[l, pl.ds(r0 + 8, C), :] * shT[0:1, ls]
            for j in range(1, 4):
                ks = ks + kf_s[l, pl.ds(r0 + 8 - j, C), :] * shT[j:j + 1, ls]
            kv = (ks * v_s[pl.ds(r0, C), ls].astype(f32)).astype(bf16)
            X_s[a, :, ls] = jnp.dot(F_s[...], kv, preferred_element_type=f32)

    def late_fwd(a0, extra=()):
        wait(cp_conv(a0, GS))
        shT = shT_s[...].astype(f32)
        _emit([(lambda a=a: fwd_chunk(a, shT)) for a in range(a0, a0 + GS)], list(extra))

    def mac_task(g, r0, l, rows, jlo, jhi, init):
        a0 = GS * g

        def run():
            rre = pl.ds(mo(r0, rows), rows)
            rim = pl.ds(mo(r0 + C, rows), rows)
            ls = slice(l * L, (l + 1) * L)
            acc = [None] * GS
            kc = {}

            def getk(d):
                if d not in kc:
                    kr = K_s[d, rre, ls]
                    ki = K_s[d, rim, ls]
                    kc[d] = (kr, ki, kr + ki)
                return kc[d]

            for j in range(jlo, jhi):
                xr = X_s[j, rre, ls]
                xi = X_s[j, rim, ls]
                xs = xr + xi
                for t in range(GS):
                    d = a0 + t - j
                    if d < 0:
                        continue
                    kr, ki, ks = getk(d)
                    terms = (kr * xr, ki * xi, ks * xs)
                    acc[t] = terms if acc[t] is None else tuple(p + s for p, s in zip(acc[t], terms))
            for t in range(GS):
                if acc[t] is None:
                    continue
                P, Q, R = acc[t]
                yr, yi = P - Q, R - P - Q
                if not init:
                    yr = yr + Z_s[a0 + t, rre, ls]
                    yi = yi + Z_s[a0 + t, rim, ls]
                Z_s[a0 + t, rre, ls] = yr
                Z_s[a0 + t, rim, ls] = yi
        return run

    def mac_tasks(g, r_base, nrows, rows, ranges, init):
        return [mac_task(g, r_base + dr, l, rows, j0, j1, init and i == 0)
                for dr in range(0, nrows, rows) for l in range(NL) for i, (j0, j1) in enumerate(ranges)]

    def mac_group(g):
        def body(i, _):
            _emit(mac_tasks(g, i * 16, 16, 16, [(0, GS * g + GS)], True))
            return 0
        jax.lax.fori_loop(0, C // 16, body, 0)

    row = jax.lax.broadcasted_iota(jnp.int32, (C, L), 0)

    def inv_task(a, l):
        def run():
            ls = slice(l * L, (l + 1) * L)
            zr = Z_s[a, 0:C, ls]
            zi = Z_s[a, C:, ls]
            if a > 0:
                sgn = jnp.where((row & 1) == 0, 1.0, -1.0).astype(f32)
                zr = zr - sgn * Z_s[a - 1, C:, ls]
                zi = zi + sgn * Z_s[a - 1, 0:C, ls]
            w = jnp.concatenate([zr, zi], axis=0).astype(bf16)
            y_s[a * C:(a + 1) * C, ls] = jnp.dot(G_s[...], w, preferred_element_type=f32)
        return run

    def inv_tasks(g):
        return [inv_task(g * GS + t, l) for t in range(GS) for l in range(NL)]

    def rep(i, rows):
        return jnp.concatenate([mod_s[i]] * (rows // 8), axis=0)

    def x1_task(r_dst, r_src):
        def run():
            q = q_s[pl.ds(r_src, RB), :].astype(f32)
            xc = q - jnp.mean(q, axis=-1, keepdims=True)
            r = jax.lax.rsqrt(jnp.mean(xc * xc, axis=-1, keepdims=True) + EPS)
            hg = (xc * r) * rep(0, RB) + rep(1, RB)
            x1_s[pl.ds(r_dst, RB), :] = hg * y_s[pl.ds(r_src, RB), :] + q
        return run

    def h2_task(r_dst, r_x1):
        def run():
            x1 = x1_s[pl.ds(r_x1, RB), :]
            xc = x1 - jnp.mean(x1, axis=-1, keepdims=True)
            r = jax.lax.rsqrt(jnp.mean(xc * xc, axis=-1, keepdims=True) + EPS)
            h2_s[pl.ds(r_dst, RB), :] = ((xc * r) * rep(2, RB) + rep(3, RB)).astype(bf16)
        return run

    def norm_tasks(r_dst, r_src, with_x1=True):
        out = []
        for t in range(BM // RB):
            a, b = mo(r_dst + t * RB, RB), mo(r_src + t * RB, RB)
            out += [x1_task(a, b), h2_task(a, a)] if with_x1 else [h2_task(a, b)]
        return out

    def silu_c():
        cc = c_s[...].astype(f32)
        return jnp.broadcast_to((cc * jax.nn.sigmoid(cc)).astype(bf16), (16, D))

    def mod_piece(sc, i):
        return jnp.dot(sc, wm_s[:, i * D:(i + 1) * D], preferred_element_type=f32)[0:8]

    def ffn_tasks(r0):
        st = {'h2': h2_s[pl.ds(r0, BM), :]}

        def gate_up(f):
            def run():
                cs = slice(f * BF, (f + 1) * BF)
                g = jnp.dot(st['h2'], wg_s[:, cs], preferred_element_type=f32)
                u = jnp.dot(st['h2'], wu_s[:, cs], preferred_element_type=f32)
                st['act'] = (jnp.maximum(g, 0.0) * u).astype(bf16)
            return run

        def down(f):
            def run():
                d = jnp.dot(st['act'], wd_s[f * BF:(f + 1) * BF, :], preferred_element_type=f32)
                st['acc'] = d if f == 0 else st['acc'] + d
            return run

        return st, [t for f in range(nf) for t in (gate_up(f), down(f))]

    def write_out(i, r0, acc):
        gb = rep(4, half)
        for h in range(2):
            rs = pl.ds(mo(r0 + h * half, half), half)
            o_s[rs, :] = (x1_s[rs, :] + gb * acc[h * half:(h + 1) * half]).astype(o_s.dtype)
            cp_o(i, h).start()

    def ffn_step(i, *others, with_x1=True):
        r0 = mo(i * BM, BM)
        st, tasks = ffn_tasks(r0)
        nxt = mo(jnp.minimum(r0 + BM, S - BM), BM)
        _emit(tasks, *others, norm_tasks(r0 + BM, nxt, with_x1))
        write_out(i, r0, st['acc'])

    wait([k0, v0, cp_F, cp_sh, cp_D, ssm0])
    shT = shT_s[...].astype(f32)
    fwd_chunk(0, shT, D_s[...].astype(f32).reshape(1, D))

    def fwd_body(a, _):
        wait(cp_conv(a, 1))
        fwd_chunk(a, shT)
        return 0
    jax.lax.fori_loop(1, 8, fwd_body, 0)

    mac_group(0)
    cp_G.wait()
    _emit(inv_tasks(0))
    mac_group(1)

    cp_c.wait()
    sc = silu_c()
    m = [None] * 5
    for i in wm_early:
        cp_wm(i).wait()
        m[i] = mod_piece(sc, i)
    sa, ca, ga, sb, cb = m
    mod_s[0] = (1.0 + ca) * ga
    mod_s[1] = sa * ga
    mod_s[2] = 1.0 + cb
    mod_s[3] = sb

    cp_q(0).wait()
    _emit(norm_tasks(0, 0))

    wait([cp_wg(0), cp_wu(0)])
    st, tasks = ffn_tasks(0)
    gu0, d0, gu1, d1, gu2, d2 = tasks
    gu0()
    cp_q(1).wait()
    _emit(inv_tasks(1), [x1_task(r, r) for r in range(BM, 2 * BM, RB)])

    def waited(copies, task):
        def run():
            wait(copies)
            task()
        return run
    wait([cp_wd(0), cp_wg(1), cp_wu(1)])
    _emit([d0, gu1, waited([cp_wd(1)], d1)], norm_tasks(BM, BM, False))
    late_fwd(8)
    wait([cp_wg(2), cp_wu(2)])
    gu2()
    wait([cp_wd(2), cp_wm(5)])
    mod_s[4] = mod_piece(silu_c(), 5)
    d2()
    write_out(0, 0, st['acc'])

    wait([cp_q(2), cp_q(3)])

    def step_a1(i, _):
        rb = (i - 1) * (C // 2)
        ffn_step(i, mac_tasks(2, rb, C // 2, 8, [(j, j + 2) for j in range(0, 12, 2)], True),
                 mac_tasks(3, rb, C // 2, 8, [(4, 6), (6, 8)], True))
        return 0
    jax.lax.fori_loop(1, 3, step_a1, 0)

    wait([cp_q(i) for i in range(4, nq)])
    chain = []
    for a in range(8, 12):
        chain += [inv_task(a, l) for l in range(NL)]
        chain += [x1_task(r, r) for r in range(a * C, (a + 1) * C, RB)]
    late_fwd(12, chain)

    def step_a2(i, _):
        rb = (i - 3) * (C // 2)
        ffn_step(i, mac_tasks(3, rb, C // 2, 8, [(0, 2), (2, 4), (8, 10), (10, 12), (12, 14), (14, 16)], False), with_x1=False)
        return 0
    jax.lax.fori_loop(3, 5, step_a2, 0)

    _emit(inv_tasks(3) + [x1_task(r, r) for r in range(12 * C, 16 * C, RB)])

    def step_b(i, _):
        ffn_step(i, with_x1=False)
        return 0
    jax.lax.fori_loop(5, nq, step_b, 0)

    wait([cp_o(i, h) for i in range(nq) for h in range(2)])


@jax.jit
def pallas_adaLN_cond__ssm_conv_h3__glu_gated_reglu__prompt_kernel(A_q, A_k, A_v, A_shift_k, A_ssm_k, A_ssm_D, B_x, B_W_gate, B_W_up, B_W_down, c, w_mod):
    del B_x
    _, S, D = A_q.shape
    Fd = B_W_gate.shape[1]
    n = S // C
    V = pltpu.VMEM
    hbm = pl.BlockSpec(memory_space=pl.ANY)
    n_sems = 5 + 3 * n + 6 + 3 * (Fd // BF) + 3 * (S // BM)
    out = pl.pallas_call(
        _kernel,
        out_shape=jax.ShapeDtypeStruct((S, D), A_q.dtype),
        in_specs=[hbm] * 13,
        out_specs=hbm,
        scratch_shapes=[
            V((4, D), bf16), V((D,), bf16), V((1, D), bf16), V((2 * C, C), bf16), V((C, 2 * C), bf16),
            V((S, D), bf16), V((S, D), bf16), V((S, D), bf16), V((D, S), bf16),
            V((D, Fd), bf16), V((D, Fd), bf16), V((Fd, D), bf16), V((D, 6 * D), bf16),
            V((D // L, S + 8, L), f32),
            V((n, 2 * C, D), f32), V((n, 2 * C, D), f32), V((n, 2 * C, D), f32),
            V((S, D), f32),
            V((S + BM, D), f32), V((S + BM, D), bf16),
            V((S, D), bf16),
            V((5, 8, D), f32),
            pltpu.SemaphoreType.DMA((n_sems,)),
        ],
        compiler_params=pltpu.CompilerParams(vmem_limit_bytes=120 * 1024 * 1024),
    )(A_q[0], A_k[0], A_v[0], A_shift_k.T, A_ssm_k, A_ssm_D, B_W_gate, B_W_up, B_W_down, c, w_mod,
      jnp.asarray(_FWD), jnp.asarray(_INV))
    return out[None]
```
